```python
import jax
import jax.numpy as jnp

def _softmax(x, axis=-1):
    return jax.nn.softmax(x, axis=axis)

def _gelu(x):
    return jax.nn.gelu(x, approximate=True)

def _silu(x):
    return jax.nn.silu(x)

def _sigmoid(x):
    return jax.nn.sigmoid(x)

def _layernorm(x, axis=-1, eps=1e-05):
    m = jnp.mean(x, axis=axis, keepdims=True)
    v = jnp.var(x, axis=axis, keepdims=True)
    return (x - m) / jnp.sqrt(v + eps)

def _scatter_add(tgt, idx, src, axis=0):
    return tgt.at[idx].add(src)

def _segment_sum(src, seg, n):
    return jax.ops.segment_sum(src, seg, n)

class _Rng:

    def __init__(self, key):
        self._k = key

    def _next(self):
        self._k, sub = jax.random.split(self._k)
        return sub

    def normal(self, shape):
        return jax.random.normal(self._next(), shape, dtype=jnp.bfloat16)

    def randint(self, lo, hi, shape):
        return jax.random.randint(self._next(), shape, lo, hi, dtype=jnp.int32)

    def uniform(self, shape, lo=0.0, hi=1.0):
        return jax.random.uniform(self._next(), shape, jnp.bfloat16, lo, hi)

    def permutation(self, n):
        return jax.random.permutation(self._next(), n)
kernel_name = 'sequential_preLN__ssm_conv_s4__mixer_gmlp__prompt'

def _fwd_setup_inputs():
    _rng = _Rng(jax.random.key(int.from_bytes(__import__("os").urandom(4), "little")))
    _w = lambda a: (lambda t: t.astype(jnp.bfloat16) if jnp.issubdtype(t.dtype, jnp.floating) else t)(jnp.asarray(a))

    def _A_setup():
        B, L, D, N = (1, 2048, 576, 128)
        A_re = -jnp.exp((lambda *s: _rng.normal(s) * 0.05)(D, N))
        A_im = jnp.pi * (lambda *s: _rng.normal(s) * 0.05)(D, N)
        B_re = (lambda *s: _rng.normal(s) * 0.05)(D, N)
        B_im = (lambda *s: _rng.normal(s) * 0.05)(D, N)
        C_re = (lambda *s: _rng.normal(s) * 0.05)(D, N)
        C_im = (lambda *s: _rng.normal(s) * 0.05)(D, N)
        log_dt = (lambda *s: _rng.normal(s) * 0.05)(D) * 0.5 - 4.0
        Dskip = (lambda *s: _rng.normal(s) * 0.05)(D)
        return {'u': _w((lambda *s: _rng.normal(s) * 0.05)(B, L, D)), 'A_re': _w(A_re), 'A_im': _w(A_im), 'B_re': _w(B_re), 'B_im': _w(B_im), 'C_re': _w(C_re), 'C_im': _w(C_im), 'log_dt': _w(log_dt), 'Dskip': _w(Dskip)}
    _A_in = _A_setup()

    def _B_setup():
        B, S, D, F = (1, 2048, 576, 4608)
        Fh = F // 2
        return {'x': _w((lambda *s: _rng.normal(s) * 0.05)(B, S, D)), 'w_in': _w((lambda *s: _rng.normal(s) * 0.05)(D, 2 * Fh)), 'w_sp': _w(0.01 * (lambda *s: _rng.normal(s) * 0.05)(S, S)), 'b_sp': _w(1.0 + 0.01 * (lambda *s: _rng.normal(s) * 0.05)(S)), 'w_out': _w((lambda *s: _rng.normal(s) * 0.05)(Fh, D))}
    _B_in = _B_setup()
    return {'A_u': _A_in['u'], 'A_A_re': _A_in['A_re'], 'A_A_im': _A_in['A_im'], 'A_B_re': _A_in['B_re'], 'A_B_im': _A_in['B_im'], 'A_C_re': _A_in['C_re'], 'A_C_im': _A_in['C_im'], 'A_log_dt': _A_in['log_dt'], 'A_Dskip': _A_in['Dskip'], 'B_x': _B_in['x'], 'B_w_in': _B_in['w_in'], 'B_w_sp': _B_in['w_sp'], 'B_b_sp': _B_in['b_sp'], 'B_w_out': _B_in['w_out']}

def _fwd_reference(A_u, A_A_re, A_A_im, A_B_re, A_B_im, A_C_re, A_C_im, A_log_dt, A_Dskip, B_x, B_w_in, B_w_sp, B_b_sp, B_w_out):

    def _A_ref(u, A_re, A_im, B_re, B_im, C_re, C_im, log_dt, Dskip):
        Bsz, L, D = u.shape
        dt = jnp.exp(log_dt)[:, None]
        A = A_re + 1j * A_im
        Bc = B_re + 1j * B_im
        Cc = C_re + 1j * C_im
        logdA = dt * A
        dB = dt * Bc
        l = (lambda x, dt: x.astype(dt))(jnp.arange(L), A_re.dtype)
        P = jnp.exp(logdA[:, :, None] * l[None, None, :])
        K = jnp.einsum('dn,dnl,dn->dl', Cc, P, dB).real
        L2 = 2 * L
        Kp = jnp.pad(K, ((0, 0), (0, L)))
        up = (lambda x, *d: x.transpose(*d))(u, 0, 2, 1)
        up = jnp.pad(up, ((0, 0), (0, 0), (0, L)))
        Kf = (lambda x, axes=(-2, -1): jnp.fft.rfft2(x.astype(jnp.float32), axes=axes))(Kp[:, None, :], axes=(-2, -1))
        Uf = (lambda x, axes=(-2, -1): jnp.fft.rfft2(x.astype(jnp.float32), axes=axes))(up[:, :, None, :], axes=(-2, -1))
        Yf = Uf * Kf[None, :, :, :]
        y = (lambda x, s, axes=(-2, -1): jnp.fft.irfft2(x, s=s, axes=axes).astype(jnp.bfloat16))(Yf, (1, L2), axes=(-2, -1))[:, :, 0, :L]
        y = (lambda x, *d: x.transpose(*d))(y, 0, 2, 1) + u * Dskip[None, None, :]
        return y

    def _B_ref(x, w_in, w_sp, b_sp, w_out):
        B, S, D = x.shape
        F = w_in.shape[-1]
        Fh = F // 2
        z = _gelu(jnp.einsum('bsd,df->bsf', x, w_in))
        z1 = z[..., :Fh].copy()
        z2 = _layernorm(z[..., Fh:], axis=-1)
        g = jnp.einsum('ts,bsf->btf', w_sp, z2) + b_sp[None, :, None]
        return jnp.einsum('bsf,fd->bsd', z1 * g, w_out)
    x = A_u
    h = x + _A_ref(_layernorm(x, axis=-1), A_A_re, A_A_im, A_B_re, A_B_im, A_C_re, A_C_im, A_log_dt, A_Dskip)
    h2 = h + _B_ref(_layernorm(h, axis=-1), B_w_in, B_w_sp, B_b_sp, B_w_out)
    return h2

def setup_inputs():
    _inp = _fwd_setup_inputs()
    _gk = jax.random.fold_in(jax.random.key(int.from_bytes(__import__("os").urandom(4), "little")), 2 ** 31 - 1)
    _shapes = [[1, 2048, 576]]
    _dtypes = ['bfloat16']
    _gks = jax.random.split(_gk, len(_shapes))
    _gs = [jax.random.normal(k, s, dtype=jnp.dtype(d)) * 0.05 for k, s, d in zip(_gks, _shapes, _dtypes)]
    _inp['grad_out'] = _gs[0]
    return _inp

def reference(A_u, A_A_re, A_A_im, A_B_re, A_B_im, A_C_re, A_C_im, A_log_dt, A_Dskip, B_w_in, B_w_sp, B_b_sp, B_w_out, B_x, grad_out):
    _const = dict(B_x=B_x)

    def _f(*_d):
        return _fwd_reference(**{'A_u': _d[0], 'A_A_re': _d[1], 'A_A_im': _d[2], 'A_B_re': _d[3], 'A_B_im': _d[4], 'A_C_re': _d[5], 'A_C_im': _d[6], 'A_log_dt': _d[7], 'A_Dskip': _d[8], 'B_w_in': _d[9], 'B_w_sp': _d[10], 'B_b_sp': _d[11], 'B_w_out': _d[12], **_const})
    _out, _vjp = jax.vjp(_f, A_u, A_A_re, A_A_im, A_B_re, A_B_im, A_C_re, A_C_im, A_log_dt, A_Dskip, B_w_in, B_w_sp, B_b_sp, B_w_out)
    _grads = _vjp(grad_out)
    _out0 = jnp.asarray(_out)
    return (_out0, *[jnp.asarray(_g) for _g in _grads])
```

```python
import math
import jax
import jax.numpy as jnp
from jax import lax
import jax.experimental.pallas as pl
import jax.experimental.pallas.tpu as pltpu

BF = jnp.bfloat16
F32 = jnp.float32
EPS = 1e-5
C = 128
TM = 128
QP = 768


def _dot(a, b):
    return jnp.dot(a, b, preferred_element_type=F32)


def _dot_tn(a, b):
    return lax.dot_general(a, b, (((0,), (0,)), ((), ())), preferred_element_type=F32)


def _dot_nt(a, b):
    return lax.dot_general(a, b, (((1,), (1,)), ((), ())), preferred_element_type=F32)


def _split(x):
    hi = x.astype(BF)
    return hi, (x - hi.astype(F32)).astype(BF)


def _dot3(fh, fl, x):
    xh, xl = _split(x)
    return _dot(fh, xh) + _dot(fh, xl) + _dot(fl, xh)


def _dot_sel(s, x):
    xh, xl = _split(x)
    xl2 = (x - xh.astype(F32) - xl.astype(F32)).astype(BF)
    return _dot(s, xh) + _dot(s, xl) + _dot(s, xl2)


def _r(x):
    return x.astype(BF).astype(F32)


def _ln(x):
    m = _r(jnp.mean(x, axis=-1, keepdims=True))
    v = _r(jnp.mean(jnp.square(x - jnp.mean(x, axis=-1, keepdims=True)), axis=-1, keepdims=True))
    sd = _r(jnp.sqrt(_r(v + EPS)))
    return _r(_r(x - m) / sd), sd


def _ln_bwd(dy, xh, sd):
    return (dy - jnp.mean(dy, axis=-1, keepdims=True)
            - xh * jnp.mean(dy * xh, axis=-1, keepdims=True)) / sd


_GC = math.sqrt(2.0 / math.pi)


def _gelu_and_grad(x):
    u = _GC * (x + 0.044715 * x * x * x)
    t = jnp.tanh(u)
    g = 0.5 * x * (1.0 + t)
    dg = 0.5 * (1.0 + t) + 0.5 * x * (1.0 - t * t) * _GC * (1.0 + 3 * 0.044715 * x * x)
    return g, dg


def _q_to_r(q):
    return jnp.where(q < 256, q, jnp.where(q < 384, 256 + 2 * (q - 256),
                     jnp.where(q < 512, 512 + 4 * (q - 384), 1024 + 8 * (q - 512))))


def _l_to_q(l):
    r = l.astype(F32).astype(BF).astype(F32).astype(jnp.int32)
    return jnp.where(r < 256, r, jnp.where(r < 512, 256 + (r - 256) // 2,
                     jnp.where(r < 1024, 384 + (r - 512) // 4, 512 + (r - 1024) // 8)))


def _seg(j):
    return 0 if j < 32 else (1 if j < 48 else (2 if j < 64 else 3))


def _kernel(x_ref, are_ref, aim_ref, bre_ref, bim_ref, cre_ref, cim_ref, ldt_ref, dsk_ref,
            win_ref, wsp_ref, bsp_ref, wout_ref, go_ref,
            out_ref, dx_ref, dare_ref, daim_ref, dbre_ref, dbim_ref, dcre_ref, dcim_ref,
            dldt_ref, ddsk_ref, dwin_ref, dwsp_ref, dbsp_ref, dwout_ref,
            xn_s, h_s, k_s, kd_s, u_s, kf_s):
    L, D = x_ref.shape
    N = are_ref.shape[0]
    NB = L // C
    NT = L // TM
    NJ = 81

    def dft(shape, kax):
        k = lax.broadcasted_iota(jnp.int32, shape, kax)
        t = lax.broadcasted_iota(jnp.int32, shape, 1 - kax)
        ang = (((2 * (k % C) + 1) * t) % (4 * C)).astype(F32) * (math.pi / (2 * C))
        return jnp.where(k < C, jnp.cos(ang), -jnp.sin(ang))
    fh, fl = _split(dft((2 * C, C), 0))
    fth, ftl = _split(dft((C, 2 * C), 1) * (1.0 / C))
    sgn = (1 - 2 * (lax.broadcasted_iota(jnp.int32, (C, 1), 0) % 2)).astype(F32)

    dt = _r(jnp.exp(ldt_ref[...].astype(F32)))

    def lam_tables(n):
        ar = are_ref[pl.ds(n, 1), :].astype(F32) * dt
        ai = aim_ref[pl.ds(n, 1), :].astype(F32) * dt
        rh = _q_to_r(8 * lax.broadcasted_iota(jnp.int32, (88, 1), 0)).astype(F32)
        jj = lax.broadcasted_iota(jnp.int32, (32, 1), 0)
        rl = ((jj % 8) << (jj // 8)).astype(F32)
        eh = jnp.exp(ar * rh); el = jnp.exp(ar * rl)
        return (eh * jnp.cos(ai * rh), eh * jnp.sin(ai * rh),
                el * jnp.cos(ai * rl), el * jnp.sin(ai * rl))

    def w_row(n):
        br = bre_ref[pl.ds(n, 1), :].astype(F32) * dt
        bi = bim_ref[pl.ds(n, 1), :].astype(F32) * dt
        cr = cre_ref[pl.ds(n, 1), :].astype(F32)
        ci = cim_ref[pl.ds(n, 1), :].astype(F32)
        return br, bi, cr, ci, cr * br - ci * bi, cr * bi + ci * br

    kd_s[...] = jnp.zeros(kd_s.shape, F32)

    def kgen(n, c):
        hr, hi, lr, li = lam_tables(n)
        _, _, _, _, wr, wi = w_row(n)
        h2r = hr * wr - hi * wi
        h2i = hr * wi + hi * wr
        for j in range(NJ):
            s = 8 * _seg(j)
            kd_s[8 * j:8 * j + 8, :] += (h2r[j:j + 1] * lr[s:s + 8] - h2i[j:j + 1] * li[s:s + 8])
        return c
    lax.fori_loop(0, N, kgen, 0)

    def kexp(i, c):
        l = i * TM + lax.broadcasted_iota(jnp.int32, (TM, QP), 0)
        q = lax.broadcasted_iota(jnp.int32, (TM, QP), 1)
        st = jnp.where(_l_to_q(l) == q, 1.0, 0.0).astype(BF)
        k_s[pl.ds(i * TM, TM), :] = _dot_sel(st, kd_s[...])
        return c
    lax.fori_loop(0, NT, kexp, 0)

    def ln1(i, c):
        r = pl.ds(i * TM, TM)
        xn_s[r, :] = (_ln(x_ref[r, :].astype(F32))[0]).astype(BF)
        return c
    lax.fori_loop(0, NT, ln1, 0)

    def tr(a, c):
        r = pl.ds(a * C, C)
        u_s[a] = _dot3(fh, fl, xn_s[r, :].astype(F32))
        kf_s[a] = _dot3(fh, fl, k_s[r, :])
        return c
    lax.fori_loop(0, NB, tr, 0)

    def fconv(a, c):
        def inner(dl, cc):
            gr, gi = cc
            b = a - dl
            bm = jnp.maximum(b - 1, 0)
            w = jnp.where(b > 0, 1.0, 0.0) * sgn
            vr = u_s[b, :C, :] - w * u_s[bm, C:, :]
            vi = u_s[b, C:, :] + w * u_s[bm, :C, :]
            kr = kf_s[dl, :C, :]; ki = kf_s[dl, C:, :]
            return gr + kr * vr - ki * vi, gi + kr * vi + ki * vr
        z0 = jnp.zeros((C, D), F32)
        gr, gi = lax.fori_loop(0, a + 1, inner, (z0, z0))
        y = _r(_dot3(fth, ftl, jnp.concatenate([gr, gi], axis=0)))
        r = pl.ds(a * C, C)
        h_s[r, :] = (_r(x_ref[r, :].astype(F32) + _r(y + _r(xn_s[r, :].astype(F32) * dsk_ref[...].astype(F32))))).astype(BF)
        return c
    lax.fori_loop(0, NB, fconv, 0)

    def gmlp(hn_s, pre_s, z2n_s, dg_s, acc2_s):
        FH = dg_s.shape[1]

        def f1(i, c):
            r = pl.ds(i * TM, TM)
            hn = _ln(h_s[r, :].astype(F32))[0].astype(BF)
            hn_s[r, :] = hn
            pre = _dot(hn, win_ref[...]).astype(BF)
            pre_s[r, :] = pre
            z2 = _r(_gelu_and_grad(pre[:, FH:].astype(F32))[0])
            z2n_s[r, :] = _ln(z2)[0].astype(BF)
            return c
        lax.fori_loop(0, NT, f1, 0)

        acc2_s[...] = jnp.zeros(acc2_s.shape, F32)

        def f2(i, c):
            r = pl.ds(i * TM, TM)
            g = _r(_r(_dot(wsp_ref[r, :], z2n_s[...])) + bsp_ref[r, :].astype(F32))
            z1, gp = _gelu_and_grad(pre_s[r, :FH].astype(F32))
            z1 = _r(z1)
            a = (z1 * g).astype(BF)
            out_ref[r, :] = (h_s[r, :].astype(F32) + _r(_dot(a, wout_ref[...]))).astype(BF)
            go = go_ref[r, :]
            acc2_s[...] += _dot_tn(a, go)
            da = _r(_dot_nt(go, wout_ref[...]))
            dg = da * z1
            dbsp_ref[r, :] = jnp.sum(dg, axis=-1, keepdims=True).astype(BF)
            dg_s[r, :] = dg.astype(BF)
            pre_s[r, :FH] = (da * g * gp).astype(BF)
            return c
        lax.fori_loop(0, NT, f2, 0)
        dwout_ref[...] = acc2_s[...].astype(BF)

        def b1(i, c):
            r = pl.ds(i * TM, TM)
            dwsp_ref[r, :] = _dot_nt(dg_s[r, :], z2n_s[...]).astype(BF)
            dz2n = _r(_dot_tn(wsp_ref[:, r], dg_s[...]))
            z, gp = _gelu_and_grad(pre_s[r, FH:].astype(F32))
            xh, sd = _ln(_r(z))
            pre_s[r, FH:] = (_ln_bwd(dz2n, xh, sd) * gp).astype(BF)
            dhn = _dot_nt(pre_s[r, :], win_ref[...])
            hh, hsd = _ln(h_s[r, :].astype(F32))
            h_s[r, :] = (_r(go_ref[r, :].astype(F32) + _ln_bwd(dhn, hh, hsd))).astype(BF)
            return c
        lax.fori_loop(0, NT, b1, 0)

        def b2(i, c):
            cs = pl.ds(pl.multiple_of(i * 512, 512), 512)
            dwin_ref[:, cs] = _dot_tn(hn_s[...], pre_s[:, cs]).astype(BF)
            return c
        lax.fori_loop(0, 2 * FH // 512, b2, 0)

    FF = win_ref.shape[1]
    pl.run_scoped(gmlp, pltpu.VMEM((L, D), BF), pltpu.VMEM((L, FF), BF),
                  pltpu.VMEM((L, FF // 2), BF), pltpu.VMEM((L, FF // 2), BF),
                  pltpu.VMEM((FF // 2, D), F32))


    def ssm_bwd(dw_s):
        def tr2(a, c):
            dh = h_s[pl.ds(a * C, C), :].astype(F32)
            dw_s[a] = _dot3(fh, fl, dh)
            return c + jnp.sum(dh * xn_s[pl.ds(a * C, C), :].astype(F32), axis=0, keepdims=True)
        ddsk_ref[...] = lax.fori_loop(0, NB, tr2, jnp.zeros((1, D), F32)).astype(BF)

        def win(a, c):
            ap = jnp.minimum(a + 1, NB - 1)
            w = jnp.where(a + 1 < NB, 1.0, 0.0) * sgn
            nr = dw_s[a, :C, :] + w * dw_s[ap, C:, :]
            ni = dw_s[a, C:, :] - w * dw_s[ap, :C, :]
            dw_s[a, :C, :] = nr
            dw_s[a, C:, :] = ni
            return c
        lax.fori_loop(0, NB, win, 0)

        def bconv(a, c):
            def inner(dl, cc):
                gr, gi, kr_, ki_ = cc
                wr_ = dw_s[a + dl, :C, :]; wi_ = dw_s[a + dl, C:, :]
                kr = kf_s[dl, :C, :]; ki = kf_s[dl, C:, :]
                ur = u_s[dl, :C, :]; ui = u_s[dl, C:, :]
                return (gr + kr * wr_ + ki * wi_, gi + kr * wi_ - ki * wr_,
                        kr_ + ur * wr_ + ui * wi_, ki_ + ur * wi_ - ui * wr_)
            z0 = jnp.zeros((C, D), F32)
            gr, gi, kr_, ki_ = lax.fori_loop(0, NB - a, inner, (z0, z0, z0, z0))
            r = pl.ds(a * C, C)
            du = _dot3(fth, ftl, jnp.concatenate([gr, gi], axis=0))
            k_s[r, :] = _dot3(fth, ftl, jnp.concatenate([kr_, ki_], axis=0))
            dh = h_s[r, :].astype(F32)
            dxn = du + dh * dsk_ref[...].astype(F32)
            xh, sd = _ln(x_ref[r, :].astype(F32))
            dx_ref[r, :] = (dh + _ln_bwd(dxn, xh, sd)).astype(BF)
            return c
        lax.fori_loop(0, NB, bconv, 0)

    pl.run_scoped(ssm_bwd, pltpu.VMEM((NB, 2 * C, D), F32))

    kd_s[...] = jnp.zeros(kd_s.shape, F32)

    def kred(i, c):
        q = lax.broadcasted_iota(jnp.int32, (QP, TM), 0)
        l = i * TM + lax.broadcasted_iota(jnp.int32, (QP, TM), 1)
        kd_s[...] += _dot_sel(jnp.where(_l_to_q(l) == q, 1.0, 0.0).astype(BF),
                              k_s[pl.ds(i * TM, TM), :])
        return c
    lax.fori_loop(0, NT, kred, 0)
    rq = _q_to_r(lax.broadcasted_iota(jnp.int32, (8, 1), 0))
    acc_dt = dldt_ref

    def pgrad(n, gdt):
        hr, hi, lr, li = lam_tables(n)
        br, bi, cr, ci, wr, wi = w_row(n)
        g1r = g1i = g2r = g2i = jnp.zeros((1, D), F32)
        for s in range(4):
            z = jnp.zeros((8, D), F32)
            a1r = a1i = a2r = a2i = z
            for j in range(NJ):
                if _seg(j) != s:
                    continue
                d1 = kd_s[8 * j:8 * j + 8, :]
                rr = _q_to_r(8 * j + lax.broadcasted_iota(jnp.int32, (8, 1), 0)).astype(F32)
                d2 = d1 * rr
                a1r = a1r + hr[j:j + 1] * d1; a1i = a1i + hi[j:j + 1] * d1
                a2r = a2r + hr[j:j + 1] * d2; a2i = a2i + hi[j:j + 1] * d2
            lr_ = lr[8 * s:8 * s + 8]; li_ = li[8 * s:8 * s + 8]
            sm = lambda v: jnp.sum(v, axis=0, keepdims=True)
            g1r = g1r + sm(a1r * lr_ - a1i * li_); g1i = g1i + sm(a1r * li_ + a1i * lr_)
            g2r = g2r + sm(a2r * lr_ - a2i * li_); g2i = g2i + sm(a2r * li_ + a2i * lr_)
        gwr, gwi = g1r, -g1i
        glr = wr * g2r - wi * g2i
        gli = -(wr * g2i + wi * g2r)
        gcr = gwr * br + gwi * bi; gci = gwi * br - gwr * bi
        gbr = gwr * cr + gwi * ci; gbi = gwi * cr - gwr * ci
        rn = pl.ds(n, 1)
        dcre_ref[rn, :] = gcr; dcim_ref[rn, :] = gci
        dbre_ref[rn, :] = (gbr * dt); dbim_ref[rn, :] = (gbi * dt)
        dare_ref[rn, :] = (glr * dt); daim_ref[rn, :] = (gli * dt)
        return gdt + gbr * br + gbi * bi + dt * (glr * are_ref[rn, :].astype(F32)
                                                 + gli * aim_ref[rn, :].astype(F32))
    acc_dt[...] = lax.fori_loop(0, N, pgrad, jnp.zeros((1, D), F32)).astype(BF)


@jax.jit
def pallas_sequential_preLN__ssm_conv_s4__mixer_gmlp__prompt_kernel(
    A_u, A_A_re, A_A_im, A_B_re, A_B_im, A_C_re, A_C_im, A_log_dt, A_Dskip,
    B_x, B_w_in, B_w_sp, B_b_sp, B_w_out, grad_out,
):
    _, L, D = A_u.shape
    N = A_A_re.shape[1]
    F = B_w_in.shape[1]
    FH = F // 2
    S = jax.ShapeDtypeStruct
    nd = S((N, D), F32)
    outs = pl.pallas_call(
        _kernel,
        out_shape=(S((L, D), BF), S((L, D), BF), nd, nd, nd, nd, nd, nd, S((1, D), BF), S((1, D), BF),
                   S((D, F), BF), S((L, L), BF), S((L, 1), BF), S((FH, D), BF)),
        scratch_shapes=[
            pltpu.VMEM((L, D), BF), pltpu.VMEM((L, D), BF),
            pltpu.VMEM((L, D), F32), pltpu.VMEM((QP, D), F32),
            pltpu.VMEM((L // C, 2 * C, D), F32), pltpu.VMEM((L // C, 2 * C, D), F32),
        ],
        compiler_params=pltpu.CompilerParams(vmem_limit_bytes=127 * 1024 * 1024),
    )(A_u[0], A_A_re.T.astype(F32), A_A_im.T.astype(F32), A_B_re.T.astype(F32), A_B_im.T.astype(F32), A_C_re.T.astype(F32), A_C_im.T.astype(F32),
      A_log_dt.reshape(1, D), A_Dskip.reshape(1, D), B_w_in, B_w_sp, B_b_sp.reshape(L, 1),
      B_w_out, grad_out[0])
    o, dx, a1, a2, b1, b2, c1, c2, dl, dd, dwi, dws, dbs, dwo = outs
    return (o[None], dx[None], a1.T.astype(BF), a2.T.astype(BF), b1.T.astype(BF), b2.T.astype(BF), c1.T.astype(BF), c2.T.astype(BF), dl.reshape(D), dd.reshape(D),
            dwi, dws, dbs.reshape(L), dwo)
```

```python
import math
import jax
import jax.numpy as jnp
from jax import lax
import jax.experimental.pallas as pl
import jax.experimental.pallas.tpu as pltpu

BF = jnp.bfloat16
F32 = jnp.float32
EPS = 1e-5
C = 128
TM = 128
QP = 768


def _dot(a, b):
    return jnp.dot(a, b, preferred_element_type=F32)


def _dot_tn(a, b):
    return lax.dot_general(a, b, (((0,), (0,)), ((), ())), preferred_element_type=F32)


def _dot_nt(a, b):
    return lax.dot_general(a, b, (((1,), (1,)), ((), ())), preferred_element_type=F32)


def _split(x):
    hi = x.astype(BF)
    return hi, (x - hi.astype(F32)).astype(BF)


def _dot3(fh, fl, x):
    xh, xl = _split(x)
    return _dot(fh, xh) + _dot(fh, xl) + _dot(fl, xh)


def _dot_sel(s, x):
    xh, xl = _split(x)
    xl2 = (x - xh.astype(F32) - xl.astype(F32)).astype(BF)
    return _dot(s, xh) + _dot(s, xl) + _dot(s, xl2)


def _r(x):
    return x.astype(BF).astype(F32)


def _ln(x):
    m = _r(jnp.mean(x, axis=-1, keepdims=True))
    v = _r(jnp.mean(jnp.square(x - jnp.mean(x, axis=-1, keepdims=True)), axis=-1, keepdims=True))
    sd = _r(jnp.sqrt(_r(v + EPS)))
    return _r(_r(x - m) / sd), sd


def _ln_bwd(dy, xh, sd):
    return (dy - jnp.mean(dy, axis=-1, keepdims=True)
            - xh * jnp.mean(dy * xh, axis=-1, keepdims=True)) / sd


_GC = math.sqrt(2.0 / math.pi)


def _gelu_and_grad(x):
    u = _GC * (x + 0.044715 * x * x * x)
    t = jnp.tanh(u)
    g = 0.5 * x * (1.0 + t)
    dg = 0.5 * (1.0 + t) + 0.5 * x * (1.0 - t * t) * _GC * (1.0 + 3 * 0.044715 * x * x)
    return g, dg


def _q_to_r(q):
    return jnp.where(q < 256, q, jnp.where(q < 384, 256 + 2 * (q - 256),
                     jnp.where(q < 512, 512 + 4 * (q - 384), 1024 + 8 * (q - 512))))


def _l_to_q(l):
    r = l.astype(F32).astype(BF).astype(F32).astype(jnp.int32)
    return jnp.where(r < 256, r, jnp.where(r < 512, 256 + (r - 256) // 2,
                     jnp.where(r < 1024, 384 + (r - 512) // 4, 512 + (r - 1024) // 8)))


def _seg(j):
    return 0 if j < 32 else (1 if j < 48 else (2 if j < 64 else 3))


def _kernel(x_ref, are_ref, aim_ref, bre_ref, bim_ref, cre_ref, cim_ref, ldt_ref, dsk_ref,
            win_ref, wsp_ref, bsp_ref, wout_ref, go_ref,
            out_ref, dx_ref, dare_ref, daim_ref, dbre_ref, dbim_ref, dcre_ref, dcim_ref,
            dldt_ref, ddsk_ref, dwin_ref, dwsp_ref, dbsp_ref, dwout_ref,
            xn_s, h_s, k_s, kd_s, u_s, kf_s):
    L, D = x_ref.shape
    N = are_ref.shape[0]
    NB = L // C
    NT = L // TM
    NJ = 81

    def dft(shape, kax):
        k = lax.broadcasted_iota(jnp.int32, shape, kax)
        t = lax.broadcasted_iota(jnp.int32, shape, 1 - kax)
        ang = (((2 * (k % C) + 1) * t) % (4 * C)).astype(F32) * (math.pi / (2 * C))
        return jnp.where(k < C, jnp.cos(ang), -jnp.sin(ang))
    fh, fl = _split(dft((2 * C, C), 0))
    fth, ftl = _split(dft((C, 2 * C), 1) * (1.0 / C))
    sgn = (1 - 2 * (lax.broadcasted_iota(jnp.int32, (C, 1), 0) % 2)).astype(F32)

    dt = _r(jnp.exp(ldt_ref[...].astype(F32)))

    SEG = ((0, 32), (32, 48), (48, 64), (64, 81))

    def cexp(r, rn=slice(None)):
        e = jnp.exp(are_ref[rn, :] * dt * r)
        th = aim_ref[rn, :] * dt * r
        return e * jnp.cos(th), e * jnp.sin(th)

    def wmat():
        br = bre_ref[...] * dt; bi = bim_ref[...] * dt
        cr = cre_ref[...]; ci = cim_ref[...]
        return cr * br - ci * bi, cr * bi + ci * br

    def fill_lo(lo_s, rn=slice(None)):
        def body(i, c):
            lo_s[0, i], lo_s[1, i] = cexp(((i % 8) << (i // 8)).astype(F32), rn)
            return c
        lax.fori_loop(0, 32, body, 0)

    kd_s[...] = jnp.zeros(kd_s.shape, F32)

    def kgen(lo_s):
        fill_lo(lo_s)
        wr, wi = wmat()
        for sg, (j0, j1) in enumerate(SEG):
            er, ei = cexp(float((0, 256, 512, 1024)[sg]))
            sr, si = cexp(float(8 << sg))

            def kg(j, c):
                hr, hi = c
                for b in range(8):
                    v = hr * lo_s[0, 8 * sg + b] - hi * lo_s[1, 8 * sg + b]
                    kd_s[pl.ds(8 * j + b, 1), :] = jnp.sum(v, axis=0, keepdims=True)
                return hr * sr - hi * si, hr * si + hi * sr
            lax.fori_loop(j0, j1, kg, (er * wr - ei * wi, er * wi + ei * wr))
    pl.run_scoped(kgen, pltpu.VMEM((2, 32, N, D), F32))

    def kexp(i, c):
        l = i * TM + lax.broadcasted_iota(jnp.int32, (TM, QP), 0)
        q = lax.broadcasted_iota(jnp.int32, (TM, QP), 1)
        st = jnp.where(_l_to_q(l) == q, 1.0, 0.0).astype(BF)
        k_s[pl.ds(i * TM, TM), :] = _dot_sel(st, kd_s[...])
        return c
    lax.fori_loop(0, NT, kexp, 0)

    def ln1(i, c):
        r = pl.ds(i * TM, TM)
        xn_s[r, :] = (_ln(x_ref[r, :].astype(F32))[0]).astype(BF)
        return c
    lax.fori_loop(0, NT, ln1, 0)

    def tr(a, c):
        r = pl.ds(a * C, C)
        u_s[a] = _dot3(fh, fl, xn_s[r, :].astype(F32))
        kf_s[a] = _dot3(fh, fl, k_s[r, :])
        return c
    lax.fori_loop(0, NB, tr, 0)

    def fconv(a, c):
        def inner(dl, cc):
            gr, gi = cc
            b = a - dl
            bm = jnp.maximum(b - 1, 0)
            w = jnp.where(b > 0, 1.0, 0.0) * sgn
            vr = u_s[b, :C, :] - w * u_s[bm, C:, :]
            vi = u_s[b, C:, :] + w * u_s[bm, :C, :]
            kr = kf_s[dl, :C, :]; ki = kf_s[dl, C:, :]
            return gr + kr * vr - ki * vi, gi + kr * vi + ki * vr
        z0 = jnp.zeros((C, D), F32)
        gr, gi = lax.fori_loop(0, a + 1, inner, (z0, z0))
        y = _r(_dot3(fth, ftl, jnp.concatenate([gr, gi], axis=0)))
        r = pl.ds(a * C, C)
        h_s[r, :] = (_r(x_ref[r, :].astype(F32) + _r(y + _r(xn_s[r, :].astype(F32) * dsk_ref[...].astype(F32))))).astype(BF)
        return c
    lax.fori_loop(0, NB, fconv, 0)

    def gmlp(pre_s, z2n_s, dg_s, acc2_s):
        FH = dg_s.shape[1]

        def f1(i, c):
            r = pl.ds(i * TM, TM)
            hn = _ln(h_s[r, :].astype(F32))[0].astype(BF)
            dx_ref[r, :] = hn
            pre = _dot(hn, win_ref[...]).astype(BF)
            pre_s[r, :] = pre
            z2 = _r(_gelu_and_grad(pre[:, FH:].astype(F32))[0])
            z2n_s[r, :] = _ln(z2)[0].astype(BF)
            return c
        lax.fori_loop(0, NT, f1, 0)

        acc2_s[...] = jnp.zeros(acc2_s.shape, F32)

        def f2(i, c):
            r = pl.ds(i * TM, TM)
            g = _r(_r(_dot(wsp_ref[r, :], z2n_s[...])) + bsp_ref[r, :].astype(F32))
            z1, gp = _gelu_and_grad(pre_s[r, :FH].astype(F32))
            z1 = _r(z1)
            a = (z1 * g).astype(BF)
            out_ref[r, :] = (h_s[r, :].astype(F32) + _r(_dot(a, wout_ref[...]))).astype(BF)
            go = go_ref[r, :]
            acc2_s[...] += _dot_tn(a, go)
            da = _r(_dot_nt(go, wout_ref[...]))
            dg = da * z1
            dbsp_ref[r, :] = jnp.sum(dg, axis=-1, keepdims=True).astype(BF)
            dg_s[r, :] = dg.astype(BF)
            pre_s[r, :FH] = (da * g * gp).astype(BF)
            return c
        lax.fori_loop(0, NT, f2, 0)
        dwout_ref[...] = acc2_s[...].astype(BF)

        def b1(i, c):
            r = pl.ds(i * TM, TM)
            dwsp_ref[r, :] = _dot_nt(dg_s[r, :], z2n_s[...]).astype(BF)
            dz2n = _r(_dot_tn(wsp_ref[:, r], dg_s[...]))
            z, gp = _gelu_and_grad(pre_s[r, FH:].astype(F32))
            xh, sd = _ln(_r(z))
            pre_s[r, FH:] = (_ln_bwd(dz2n, xh, sd) * gp).astype(BF)
            dhn = _dot_nt(pre_s[r, :], win_ref[...])
            hh, hsd = _ln(h_s[r, :].astype(F32))
            h_s[r, :] = (_r(go_ref[r, :].astype(F32) + _ln_bwd(dhn, hh, hsd))).astype(BF)
            return c
        lax.fori_loop(0, NT, b1, 0)

        def b2(i, c):
            cs = pl.ds(pl.multiple_of(i * 512, 512), 512)
            dwin_ref[:, cs] = _dot_tn(dx_ref[...], pre_s[:, cs]).astype(BF)
            return c
        lax.fori_loop(0, 2 * FH // 512, b2, 0)

    FF = win_ref.shape[1]
    pl.run_scoped(gmlp, pltpu.VMEM((L, FF), BF),
                  pltpu.VMEM((L, FF // 2), BF), pltpu.VMEM((L, FF // 2), BF),
                  pltpu.VMEM((FF // 2, D), F32))


    def ssm_bwd(dw_s):
        def tr2(a, c):
            dh = h_s[pl.ds(a * C, C), :].astype(F32)
            dw_s[a] = _dot3(fh, fl, dh)
            return c + jnp.sum(dh * xn_s[pl.ds(a * C, C), :].astype(F32), axis=0, keepdims=True)
        ddsk_ref[...] = lax.fori_loop(0, NB, tr2, jnp.zeros((1, D), F32)).astype(BF)

        def win(a, c):
            ap = jnp.minimum(a + 1, NB - 1)
            w = jnp.where(a + 1 < NB, 1.0, 0.0) * sgn
            nr = dw_s[a, :C, :] + w * dw_s[ap, C:, :]
            ni = dw_s[a, C:, :] - w * dw_s[ap, :C, :]
            dw_s[a, :C, :] = nr
            dw_s[a, C:, :] = ni
            return c
        lax.fori_loop(0, NB, win, 0)

        def bconv(a, c):
            def inner(dl, cc):
                gr, gi, kr_, ki_ = cc
                wr_ = dw_s[a + dl, :C, :]; wi_ = dw_s[a + dl, C:, :]
                kr = kf_s[dl, :C, :]; ki = kf_s[dl, C:, :]
                ur = u_s[dl, :C, :]; ui = u_s[dl, C:, :]
                return (gr + kr * wr_ + ki * wi_, gi + kr * wi_ - ki * wr_,
                        kr_ + ur * wr_ + ui * wi_, ki_ + ur * wi_ - ui * wr_)
            z0 = jnp.zeros((C, D), F32)
            gr, gi, kr_, ki_ = lax.fori_loop(0, NB - a, inner, (z0, z0, z0, z0))
            r = pl.ds(a * C, C)
            du = _dot3(fth, ftl, jnp.concatenate([gr, gi], axis=0))
            k_s[r, :] = _dot3(fth, ftl, jnp.concatenate([kr_, ki_], axis=0))
            dh = h_s[r, :].astype(F32)
            dxn = du + dh * dsk_ref[...].astype(F32)
            xh, sd = _ln(x_ref[r, :].astype(F32))
            dx_ref[r, :] = (dh + _ln_bwd(dxn, xh, sd)).astype(BF)
            return c
        lax.fori_loop(0, NB, bconv, 0)

    pl.run_scoped(ssm_bwd, pltpu.VMEM((NB, 2 * C, D), F32))

    kd_s[...] = jnp.zeros(kd_s.shape, F32)

    def kred(i, c):
        q = lax.broadcasted_iota(jnp.int32, (QP, TM), 0)
        l = i * TM + lax.broadcasted_iota(jnp.int32, (QP, TM), 1)
        kd_s[...] += _dot_sel(jnp.where(_l_to_q(l) == q, 1.0, 0.0).astype(BF),
                              k_s[pl.ds(i * TM, TM), :])
        return c
    lax.fori_loop(0, NT, kred, 0)
    def pgrad(lo_s):
        def chunk(nc, c0):
            rn = pl.ds(pl.multiple_of(nc * 16, 16), 16)
            fill_lo(lo_s, rn)
            z = jnp.zeros((16, D), F32)
            g = (z, z, z, z)
            for sg, (j0, j1) in enumerate(SEG):
                sr, si = cexp(float(8 << sg), rn)

                def pg(j, c):
                    hr, hi, g1r, g1i, g2r, g2i = c
                    t1r = t1i = t2r = t2i = z
                    for b in range(8):
                        d1 = kd_s[pl.ds(8 * j + b, 1), :]
                        d2 = d1 * float(b << sg)
                        lr = lo_s[0, 8 * sg + b]; li = lo_s[1, 8 * sg + b]
                        t1r = t1r + d1 * lr; t1i = t1i + d1 * li
                        t2r = t2r + d2 * lr; t2i = t2i + d2 * li
                    rh = _q_to_r(8 * j).astype(F32)
                    t2r = t2r + rh * t1r; t2i = t2i + rh * t1i
                    return (hr * sr - hi * si, hr * si + hi * sr,
                            g1r + hr * t1r - hi * t1i, g1i + hr * t1i + hi * t1r,
                            g2r + hr * t2r - hi * t2i, g2i + hr * t2i + hi * t2r)
                g = lax.fori_loop(j0, j1, pg, cexp(float((0, 256, 512, 1024)[sg]), rn) + tuple(g))[2:]
            dare_ref[rn, :], daim_ref[rn, :], dbre_ref[rn, :], dbim_ref[rn, :] = g
            return c0
        lax.fori_loop(0, N // 16, chunk, 0)
        g = (dare_ref[...], daim_ref[...], dbre_ref[...], dbim_ref[...])
        g1r, g1i, g2r, g2i = g
        wr, wi = wmat()
        br = bre_ref[...] * dt; bi = bim_ref[...] * dt
        cr = cre_ref[...]; ci = cim_ref[...]
        gwr, gwi = g1r, -g1i
        glr = wr * g2r - wi * g2i
        gli = -(wr * g2i + wi * g2r)
        gbr = gwr * cr + gwi * ci; gbi = gwi * cr - gwr * ci
        dcre_ref[...] = gwr * br + gwi * bi; dcim_ref[...] = gwi * br - gwr * bi
        dbre_ref[...] = gbr * dt; dbim_ref[...] = gbi * dt
        dare_ref[...] = glr * dt; daim_ref[...] = gli * dt
        dldt_ref[...] = jnp.sum(gbr * br + gbi * bi + dt * (glr * are_ref[...] + gli * aim_ref[...]),
                                axis=0, keepdims=True).astype(BF)
    pl.run_scoped(pgrad, pltpu.VMEM((2, 32, 16, D), F32))


@jax.jit
def pallas_sequential_preLN__ssm_conv_s4__mixer_gmlp__prompt_kernel(
    A_u, A_A_re, A_A_im, A_B_re, A_B_im, A_C_re, A_C_im, A_log_dt, A_Dskip,
    B_x, B_w_in, B_w_sp, B_b_sp, B_w_out, grad_out,
):
    _, L, D = A_u.shape
    N = A_A_re.shape[1]
    F = B_w_in.shape[1]
    FH = F // 2
    S = jax.ShapeDtypeStruct
    nd = S((N, D), F32)
    outs = pl.pallas_call(
        _kernel,
        out_shape=(S((L, D), BF), S((L, D), BF), nd, nd, nd, nd, nd, nd, S((1, D), BF), S((1, D), BF),
                   S((D, F), BF), S((L, L), BF), S((L, 1), BF), S((FH, D), BF)),
        scratch_shapes=[
            pltpu.VMEM((L, D), BF), pltpu.VMEM((L, D), BF),
            pltpu.VMEM((L, D), F32), pltpu.VMEM((QP, D), F32),
            pltpu.VMEM((L // C, 2 * C, D), F32), pltpu.VMEM((L // C, 2 * C, D), F32),
        ],
        compiler_params=pltpu.CompilerParams(vmem_limit_bytes=127 * 1024 * 1024),
    )(A_u[0], A_A_re.T.astype(F32), A_A_im.T.astype(F32), A_B_re.T.astype(F32), A_B_im.T.astype(F32), A_C_re.T.astype(F32), A_C_im.T.astype(F32),
      A_log_dt.reshape(1, D), A_Dskip.reshape(1, D), B_w_in, B_w_sp, B_b_sp.reshape(L, 1),
      B_w_out, grad_out[0])
    o, dx, a1, a2, b1, b2, c1, c2, dl, dd, dwi, dws, dbs, dwo = outs
    return (o[None], dx[None], a1.T.astype(BF), a2.T.astype(BF), b1.T.astype(BF), b2.T.astype(BF), c1.T.astype(BF), c2.T.astype(BF), dl.reshape(D), dd.reshape(D),
            dwi, dws, dbs.reshape(L), dwo)
```

```python
import math
import jax
import jax.numpy as jnp
from jax import lax
import jax.experimental.pallas as pl
import jax.experimental.pallas.tpu as pltpu

BF = jnp.bfloat16
F32 = jnp.float32
EPS = 1e-5
C = 128
TM = 128
QP = 768


def _dot(a, b):
    return jnp.dot(a, b, preferred_element_type=F32)


def _dot_tn(a, b):
    return lax.dot_general(a, b, (((0,), (0,)), ((), ())), preferred_element_type=F32)


def _dot_nt(a, b):
    return lax.dot_general(a, b, (((1,), (1,)), ((), ())), preferred_element_type=F32)


def _split(x):
    hi = x.astype(BF)
    return hi, (x - hi.astype(F32)).astype(BF)


def _dot3(fh, fl, x):
    xh, xl = _split(x)
    return _dot(fh, xh) + _dot(fh, xl) + _dot(fl, xh)


def _dot_sel(s, x):
    xh, xl = _split(x)
    xl2 = (x - xh.astype(F32) - xl.astype(F32)).astype(BF)
    return _dot(s, xh) + _dot(s, xl) + _dot(s, xl2)


def _r(x):
    return x.astype(BF).astype(F32)


def _ln(x):
    m = _r(jnp.mean(x, axis=-1, keepdims=True))
    v = _r(jnp.mean(jnp.square(x - jnp.mean(x, axis=-1, keepdims=True)), axis=-1, keepdims=True))
    sd = _r(jnp.sqrt(_r(v + EPS)))
    return _r(_r(x - m) / sd), sd


def _ln_bwd(dy, xh, sd):
    return (dy - jnp.mean(dy, axis=-1, keepdims=True)
            - xh * jnp.mean(dy * xh, axis=-1, keepdims=True)) / sd


_GC = math.sqrt(2.0 / math.pi)


def _gelu_and_grad(x):
    u = _GC * (x + 0.044715 * x * x * x)
    t = jnp.tanh(u)
    g = 0.5 * x * (1.0 + t)
    dg = 0.5 * (1.0 + t) + 0.5 * x * (1.0 - t * t) * _GC * (1.0 + 3 * 0.044715 * x * x)
    return g, dg


def _q_to_r(q):
    return jnp.where(q < 256, q, jnp.where(q < 384, 256 + 2 * (q - 256),
                     jnp.where(q < 512, 512 + 4 * (q - 384), 1024 + 8 * (q - 512))))


def _l_to_q(l):
    r = l.astype(F32).astype(BF).astype(F32).astype(jnp.int32)
    return jnp.where(r < 256, r, jnp.where(r < 512, 256 + (r - 256) // 2,
                     jnp.where(r < 1024, 384 + (r - 512) // 4, 512 + (r - 1024) // 8)))


def _seg(j):
    return 0 if j < 32 else (1 if j < 48 else (2 if j < 64 else 3))


def _kernel(x_ref, are_ref, aim_ref, bre_ref, bim_ref, cre_ref, cim_ref, ldt_ref, dsk_ref,
            win_ref, wsp_ref, bsp_ref, wout_ref, go_ref,
            out_ref, dx_ref, dare_ref, daim_ref, dbre_ref, dbim_ref, dcre_ref, dcim_ref,
            dldt_ref, ddsk_ref, dwin_ref, dwsp_ref, dbsp_ref, dwout_ref,
            xn_s, h_s, k_s, kd_s, u_s, kf_s):
    L, D = x_ref.shape
    N = are_ref.shape[0]
    NB = L // C
    NT = L // TM
    NJ = 81

    def dft(shape, kax):
        k = lax.broadcasted_iota(jnp.int32, shape, kax)
        t = lax.broadcasted_iota(jnp.int32, shape, 1 - kax)
        ang = (((2 * (k % C) + 1) * t) % (4 * C)).astype(F32) * (math.pi / (2 * C))
        return jnp.where(k < C, jnp.cos(ang), -jnp.sin(ang))
    fh, fl = _split(dft((2 * C, C), 0))
    fth, ftl = _split(dft((C, 2 * C), 1) * (1.0 / C))
    sgn = (1 - 2 * (lax.broadcasted_iota(jnp.int32, (C, 1), 0) % 2)).astype(F32)

    dt = _r(jnp.exp(ldt_ref[...].astype(F32)))

    SEG = ((0, 32), (32, 48), (48, 64), (64, 81))

    def cexp(r, rn=slice(None)):
        e = jnp.exp(are_ref[rn, :] * dt * r)
        th = aim_ref[rn, :] * dt * r
        return e * jnp.cos(th), e * jnp.sin(th)

    def wmat():
        br = bre_ref[...] * dt; bi = bim_ref[...] * dt
        cr = cre_ref[...]; ci = cim_ref[...]
        return cr * br - ci * bi, cr * bi + ci * br

    def fill_lo(lo_s, rn=slice(None)):
        er, ei = cexp(1.0, rn)
        for sg in range(4):
            pr = jnp.ones_like(er); pi_ = jnp.zeros_like(er)
            for b in range(8):
                lo_s[0, 8 * sg + b] = pr; lo_s[1, 8 * sg + b] = pi_
                pr, pi_ = pr * er - pi_ * ei, pr * ei + pi_ * er
            er, ei = er * er - ei * ei, 2.0 * er * ei

    kd_s[...] = jnp.zeros(kd_s.shape, F32)

    def kgen(lo_s):
        fill_lo(lo_s)
        wr, wi = wmat()
        for sg, (j0, j1) in enumerate(SEG):
            er, ei = cexp(float((0, 256, 512, 1024)[sg]))
            sr, si = cexp(float(8 << sg))

            def kg(j, c):
                hr, hi = c
                for b in range(8):
                    v = hr * lo_s[0, 8 * sg + b] - hi * lo_s[1, 8 * sg + b]
                    kd_s[pl.ds(8 * j + b, 1), :] = jnp.sum(v, axis=0, keepdims=True)
                return hr * sr - hi * si, hr * si + hi * sr
            lax.fori_loop(j0, j1, kg, (er * wr - ei * wi, er * wi + ei * wr))
    pl.run_scoped(kgen, pltpu.VMEM((2, 32, N, D), F32))

    def kexp(i, c):
        l = i * TM + lax.broadcasted_iota(jnp.int32, (TM, QP), 0)
        q = lax.broadcasted_iota(jnp.int32, (TM, QP), 1)
        st = jnp.where(_l_to_q(l) == q, 1.0, 0.0).astype(BF)
        k_s[pl.ds(i * TM, TM), :] = _dot_sel(st, kd_s[...])
        return c
    lax.fori_loop(0, NT, kexp, 0)

    def ln1(i, c):
        r = pl.ds(i * TM, TM)
        xn_s[r, :] = (_ln(x_ref[r, :].astype(F32))[0]).astype(BF)
        return c
    lax.fori_loop(0, NT, ln1, 0)

    def tr(a, c):
        r = pl.ds(a * C, C)
        u_s[a] = _dot3(fh, fl, xn_s[r, :].astype(F32))
        kf_s[a] = _dot3(fh, fl, k_s[r, :])
        return c
    lax.fori_loop(0, NB, tr, 0)

    def fconv(a, c):
        GR, GI = [], []
        for k0 in range(0, C, 32):
            re = slice(k0, k0 + 32); im = slice(C + k0, C + k0 + 32)

            def inner(dl, cc):
                gr, gi = cc
                b = a - dl
                bm = jnp.maximum(b - 1, 0)
                w = jnp.where(b > 0, 1.0, 0.0) * sgn[:32]
                vr = u_s[b, re, :] - w * u_s[bm, im, :]
                vi = u_s[b, im, :] + w * u_s[bm, re, :]
                kr = kf_s[dl, re, :]; ki = kf_s[dl, im, :]
                return gr + kr * vr - ki * vi, gi + kr * vi + ki * vr
            z0 = jnp.zeros((32, D), F32)
            gr, gi = lax.fori_loop(0, a + 1, inner, (z0, z0))
            GR.append(gr); GI.append(gi)
        y = _r(_dot3(fth, ftl, jnp.concatenate(GR + GI, axis=0)))
        r = pl.ds(a * C, C)
        h_s[r, :] = (_r(x_ref[r, :].astype(F32) + _r(y + _r(xn_s[r, :].astype(F32) * dsk_ref[...].astype(F32))))).astype(BF)
        return c
    lax.fori_loop(0, NB, fconv, 0)

    def gmlp(pre_s, z2n_s, dg_s, acc2_s):
        FH = dg_s.shape[1]

        def f1(i, c):
            r = pl.ds(i * TM, TM)
            hn = _ln(h_s[r, :].astype(F32))[0].astype(BF)
            dx_ref[r, :] = hn
            pre = _dot(hn, win_ref[...]).astype(BF)
            pre_s[r, :] = pre
            z2 = _r(_gelu_and_grad(pre[:, FH:].astype(F32))[0])
            z2n_s[r, :] = _ln(z2)[0].astype(BF)
            return c
        lax.fori_loop(0, NT, f1, 0)

        acc2_s[...] = jnp.zeros(acc2_s.shape, F32)

        def f2(i, c):
            r = pl.ds(i * TM, TM)
            g = _r(_r(_dot(wsp_ref[r, :], z2n_s[...])) + bsp_ref[r, :].astype(F32))
            z1, gp = _gelu_and_grad(pre_s[r, :FH].astype(F32))
            z1 = _r(z1)
            a = (z1 * g).astype(BF)
            out_ref[r, :] = (h_s[r, :].astype(F32) + _r(_dot(a, wout_ref[...]))).astype(BF)
            go = go_ref[r, :]
            acc2_s[...] += _dot_tn(a, go)
            da = _r(_dot_nt(go, wout_ref[...]))
            dg = da * z1
            dbsp_ref[r, :] = jnp.sum(dg, axis=-1, keepdims=True).astype(BF)
            dg_s[r, :] = dg.astype(BF)
            pre_s[r, :FH] = (da * g * gp).astype(BF)
            return c
        lax.fori_loop(0, NT, f2, 0)
        dwout_ref[...] = acc2_s[...].astype(BF)

        def b1(i, c):
            r = pl.ds(i * TM, TM)
            dwsp_ref[r, :] = _dot_nt(dg_s[r, :], z2n_s[...]).astype(BF)
            dz2n = _r(_dot_tn(wsp_ref[:, r], dg_s[...]))
            z, gp = _gelu_and_grad(pre_s[r, FH:].astype(F32))
            xh, sd = _ln(_r(z))
            pre_s[r, FH:] = (_ln_bwd(dz2n, xh, sd) * gp).astype(BF)
            dhn = _dot_nt(pre_s[r, :], win_ref[...])
            hh, hsd = _ln(h_s[r, :].astype(F32))
            h_s[r, :] = (_r(go_ref[r, :].astype(F32) + _ln_bwd(dhn, hh, hsd))).astype(BF)
            return c
        lax.fori_loop(0, NT, b1, 0)

        def b2(i, c):
            cs = pl.ds(pl.multiple_of(i * 512, 512), 512)
            dwin_ref[:, cs] = _dot_tn(dx_ref[...], pre_s[:, cs]).astype(BF)
            return c
        lax.fori_loop(0, 2 * FH // 512, b2, 0)

    FF = win_ref.shape[1]
    pl.run_scoped(gmlp, pltpu.VMEM((L, FF), BF),
                  pltpu.VMEM((L, FF // 2), BF), pltpu.VMEM((L, FF // 2), BF),
                  pltpu.VMEM((FF // 2, D), F32))


    def ssm_bwd(dw_s):
        def tr2(a, c):
            dh = h_s[pl.ds(a * C, C), :].astype(F32)
            dw_s[a] = _dot3(fh, fl, dh)
            return c + jnp.sum(dh * xn_s[pl.ds(a * C, C), :].astype(F32), axis=0, keepdims=True)
        ddsk_ref[...] = lax.fori_loop(0, NB, tr2, jnp.zeros((1, D), F32)).astype(BF)

        def win(a, c):
            ap = jnp.minimum(a + 1, NB - 1)
            w = jnp.where(a + 1 < NB, 1.0, 0.0) * sgn
            nr = dw_s[a, :C, :] + w * dw_s[ap, C:, :]
            ni = dw_s[a, C:, :] - w * dw_s[ap, :C, :]
            dw_s[a, :C, :] = nr
            dw_s[a, C:, :] = ni
            return c
        lax.fori_loop(0, NB, win, 0)

        def bconv(a, c):
            acc = [[], [], [], []]
            for k0 in range(0, C, 16):
                re = slice(k0, k0 + 16); im = slice(C + k0, C + k0 + 16)

                def inner(dl, cc):
                    gr, gi, kr_, ki_ = cc
                    wr_ = dw_s[a + dl, re, :]; wi_ = dw_s[a + dl, im, :]
                    kr = kf_s[dl, re, :]; ki = kf_s[dl, im, :]
                    ur = u_s[dl, re, :]; ui = u_s[dl, im, :]
                    return (gr + kr * wr_ + ki * wi_, gi + kr * wi_ - ki * wr_,
                            kr_ + ur * wr_ + ui * wi_, ki_ + ur * wi_ - ui * wr_)
                z0 = jnp.zeros((16, D), F32)
                for lst, v in zip(acc, lax.fori_loop(0, NB - a, inner, (z0, z0, z0, z0))):
                    lst.append(v)
            r = pl.ds(a * C, C)
            du = _dot3(fth, ftl, jnp.concatenate(acc[0] + acc[1], axis=0))
            k_s[r, :] = _dot3(fth, ftl, jnp.concatenate(acc[2] + acc[3], axis=0))
            dh = h_s[r, :].astype(F32)
            dxn = du + dh * dsk_ref[...].astype(F32)
            xh, sd = _ln(x_ref[r, :].astype(F32))
            dx_ref[r, :] = (dh + _ln_bwd(dxn, xh, sd)).astype(BF)
            return c
        lax.fori_loop(0, NB, bconv, 0)

    pl.run_scoped(ssm_bwd, pltpu.VMEM((NB, 2 * C, D), F32))

    kd_s[...] = jnp.zeros(kd_s.shape, F32)

    def kred(i, c):
        q = lax.broadcasted_iota(jnp.int32, (QP, TM), 0)
        l = i * TM + lax.broadcasted_iota(jnp.int32, (QP, TM), 1)
        kd_s[...] += _dot_sel(jnp.where(_l_to_q(l) == q, 1.0, 0.0).astype(BF),
                              k_s[pl.ds(i * TM, TM), :])
        return c
    lax.fori_loop(0, NT, kred, 0)
    def pgrad(lo_s):
        def chunk(nc, c0):
            rn = pl.ds(pl.multiple_of(nc * 16, 16), 16)
            fill_lo(lo_s, rn)
            z = jnp.zeros((16, D), F32)
            g = (z, z, z, z)
            for sg, (j0, j1) in enumerate(SEG):
                sr, si = cexp(float(8 << sg), rn)

                def pg(j, c):
                    hr, hi, g1r, g1i, g2r, g2i = c
                    t1r = t1i = t2r = t2i = z
                    for b in range(8):
                        d1 = kd_s[pl.ds(8 * j + b, 1), :]
                        d2 = d1 * float(b << sg)
                        lr = lo_s[0, 8 * sg + b]; li = lo_s[1, 8 * sg + b]
                        t1r = t1r + d1 * lr; t1i = t1i + d1 * li
                        t2r = t2r + d2 * lr; t2i = t2i + d2 * li
                    rh = _q_to_r(8 * j).astype(F32)
                    t2r = t2r + rh * t1r; t2i = t2i + rh * t1i
                    return (hr * sr - hi * si, hr * si + hi * sr,
                            g1r + hr * t1r - hi * t1i, g1i + hr * t1i + hi * t1r,
                            g2r + hr * t2r - hi * t2i, g2i + hr * t2i + hi * t2r)
                g = lax.fori_loop(j0, j1, pg, cexp(float((0, 256, 512, 1024)[sg]), rn) + tuple(g))[2:]
            dare_ref[rn, :], daim_ref[rn, :], dbre_ref[rn, :], dbim_ref[rn, :] = g
            return c0
        lax.fori_loop(0, N // 16, chunk, 0)
        g = (dare_ref[...], daim_ref[...], dbre_ref[...], dbim_ref[...])
        g1r, g1i, g2r, g2i = g
        wr, wi = wmat()
        br = bre_ref[...] * dt; bi = bim_ref[...] * dt
        cr = cre_ref[...]; ci = cim_ref[...]
        gwr, gwi = g1r, -g1i
        glr = wr * g2r - wi * g2i
        gli = -(wr * g2i + wi * g2r)
        gbr = gwr * cr + gwi * ci; gbi = gwi * cr - gwr * ci
        dcre_ref[...] = gwr * br + gwi * bi; dcim_ref[...] = gwi * br - gwr * bi
        dbre_ref[...] = gbr * dt; dbim_ref[...] = gbi * dt
        dare_ref[...] = glr * dt; daim_ref[...] = gli * dt
        dldt_ref[...] = jnp.sum(gbr * br + gbi * bi + dt * (glr * are_ref[...] + gli * aim_ref[...]),
                                axis=0, keepdims=True).astype(BF)
    pl.run_scoped(pgrad, pltpu.VMEM((2, 32, 16, D), F32))


@jax.jit
def pallas_sequential_preLN__ssm_conv_s4__mixer_gmlp__prompt_kernel(
    A_u, A_A_re, A_A_im, A_B_re, A_B_im, A_C_re, A_C_im, A_log_dt, A_Dskip,
    B_x, B_w_in, B_w_sp, B_b_sp, B_w_out, grad_out,
):
    _, L, D = A_u.shape
    N = A_A_re.shape[1]
    F = B_w_in.shape[1]
    FH = F // 2
    S = jax.ShapeDtypeStruct
    nd = S((N, D), F32)
    outs = pl.pallas_call(
        _kernel,
        out_shape=(S((L, D), BF), S((L, D), BF), nd, nd, nd, nd, nd, nd, S((1, D), BF), S((1, D), BF),
                   S((D, F), BF), S((L, L), BF), S((L, 1), BF), S((FH, D), BF)),
        scratch_shapes=[
            pltpu.VMEM((L, D), BF), pltpu.VMEM((L, D), BF),
            pltpu.VMEM((L, D), F32), pltpu.VMEM((QP, D), F32),
            pltpu.VMEM((L // C, 2 * C, D), F32), pltpu.VMEM((L // C, 2 * C, D), F32),
        ],
        compiler_params=pltpu.CompilerParams(vmem_limit_bytes=127 * 1024 * 1024),
    )(A_u[0], A_A_re.T.astype(F32), A_A_im.T.astype(F32), A_B_re.T.astype(F32), A_B_im.T.astype(F32), A_C_re.T.astype(F32), A_C_im.T.astype(F32),
      A_log_dt.reshape(1, D), A_Dskip.reshape(1, D), B_w_in, B_w_sp, B_b_sp.reshape(L, 1),
      B_w_out, grad_out[0])
    o, dx, a1, a2, b1, b2, c1, c2, dl, dd, dwi, dws, dbs, dwo = outs
    return (o[None], dx[None], a1.T.astype(BF), a2.T.astype(BF), b1.T.astype(BF), b2.T.astype(BF), c1.T.astype(BF), c2.T.astype(BF), dl.reshape(D), dd.reshape(D),
            dwi, dws, dbs.reshape(L), dwo)
```

```python
import math
import jax
import jax.numpy as jnp
from jax import lax
import jax.experimental.pallas as pl
import jax.experimental.pallas.tpu as pltpu

BF = jnp.bfloat16
F32 = jnp.float32
EPS = 1e-5
C = 128
TM = 128
QP = 768


def _dot(a, b):
    return jnp.dot(a, b, preferred_element_type=F32)


def _dot_tn(a, b):
    return lax.dot_general(a, b, (((0,), (0,)), ((), ())), preferred_element_type=F32)


def _dot_nt(a, b):
    return lax.dot_general(a, b, (((1,), (1,)), ((), ())), preferred_element_type=F32)


def _split(x):
    hi = x.astype(BF)
    return hi, (x - hi.astype(F32)).astype(BF)


def _dot3(fh, fl, x):
    xh, xl = _split(x)
    return _dot(fh, xh) + _dot(fh, xl) + _dot(fl, xh)


def _dot_sel(s, x):
    xh, xl = _split(x)
    xl2 = (x - xh.astype(F32) - xl.astype(F32)).astype(BF)
    return _dot(s, xh) + _dot(s, xl) + _dot(s, xl2)


def _r(x):
    return x.astype(BF).astype(F32)


def _ln(x):
    m = _r(jnp.mean(x, axis=-1, keepdims=True))
    v = _r(jnp.mean(jnp.square(x - jnp.mean(x, axis=-1, keepdims=True)), axis=-1, keepdims=True))
    sd = _r(jnp.sqrt(_r(v + EPS)))
    return _r(_r(x - m) / sd), sd


def _ln_bwd(dy, xh, sd):
    return (dy - jnp.mean(dy, axis=-1, keepdims=True)
            - xh * jnp.mean(dy * xh, axis=-1, keepdims=True)) / sd


_GC = math.sqrt(2.0 / math.pi)


def _gelu_and_grad(x):
    u = _GC * (x + 0.044715 * x * x * x)
    t = jnp.tanh(u)
    g = 0.5 * x * (1.0 + t)
    dg = 0.5 * (1.0 + t) + 0.5 * x * (1.0 - t * t) * _GC * (1.0 + 3 * 0.044715 * x * x)
    return g, dg


def _q_to_r(q):
    return jnp.where(q < 256, q, jnp.where(q < 384, 256 + 2 * (q - 256),
                     jnp.where(q < 512, 512 + 4 * (q - 384), 1024 + 8 * (q - 512))))


def _l_to_q(l):
    r = l.astype(F32).astype(BF).astype(F32).astype(jnp.int32)
    return jnp.where(r < 256, r, jnp.where(r < 512, 256 + (r - 256) // 2,
                     jnp.where(r < 1024, 384 + (r - 512) // 4, 512 + (r - 1024) // 8)))


def _seg(j):
    return 0 if j < 32 else (1 if j < 48 else (2 if j < 64 else 3))


def _kernel(x_ref, are_ref, aim_ref, bre_ref, bim_ref, cre_ref, cim_ref, ldt_ref, dsk_ref,
            win_ref, wsp_ref, bsp_ref, wout_ref, go_ref,
            out_ref, dx_ref, dare_ref, daim_ref, dbre_ref, dbim_ref, dcre_ref, dcim_ref,
            dldt_ref, ddsk_ref, dwin_ref, dwsp_ref, dbsp_ref, dwout_ref,
            xn_s, h_s, k_s, kd_s, u_s, kf_s):
    L, D = x_ref.shape
    N = are_ref.shape[0]
    NB = L // C
    NT = L // TM
    NJ = 81

    def dft(shape, kax):
        k = lax.broadcasted_iota(jnp.int32, shape, kax)
        t = lax.broadcasted_iota(jnp.int32, shape, 1 - kax)
        ang = (((2 * (k % C) + 1) * t) % (4 * C)).astype(F32) * (math.pi / (2 * C))
        return jnp.where(k < C, jnp.cos(ang), -jnp.sin(ang))
    fh, fl = _split(dft((2 * C, C), 0))
    fth, ftl = _split(dft((C, 2 * C), 1) * (1.0 / C))
    sgn = (1 - 2 * (lax.broadcasted_iota(jnp.int32, (C, 1), 0) % 2)).astype(F32)

    dt = _r(jnp.exp(ldt_ref[...].astype(F32)))

    SEG = ((0, 32), (32, 48), (48, 64), (64, 81))

    def cexp(r, rn=slice(None)):
        e = jnp.exp(are_ref[rn, :] * dt * r)
        th = aim_ref[rn, :] * dt * r
        return e * jnp.cos(th), e * jnp.sin(th)

    def wmat(rn=slice(None)):
        br = bre_ref[rn, :] * dt; bi = bim_ref[rn, :] * dt
        cr = cre_ref[rn, :]; ci = cim_ref[rn, :]
        return cr * br - ci * bi, cr * bi + ci * br

    def fill_lo(lo_s, rn=slice(None)):
        er, ei = cexp(1.0, rn)
        for sg in range(4):
            pr = jnp.ones_like(er); pi_ = jnp.zeros_like(er)
            for b in range(8):
                lo_s[0, 8 * sg + b] = pr; lo_s[1, 8 * sg + b] = pi_
                pr, pi_ = pr * er - pi_ * ei, pr * ei + pi_ * er
            er, ei = er * er - ei * ei, 2.0 * er * ei

    kd_s[...] = jnp.zeros(kd_s.shape, F32)

    def kgen(lo_s, kp_s):
        kp_s[...] = jnp.zeros(kp_s.shape, F32)

        def kchunk(nc, c0):
            rn = pl.ds(pl.multiple_of(nc * 16, 16), 16)
            fill_lo(lo_s, rn)
            wr, wi = wmat(rn)
            for sg, (j0, j1) in enumerate(SEG):
                er, ei = cexp(float((0, 256, 512, 1024)[sg]), rn)
                sr, si = cexp(float(8 << sg), rn)

                def kg(j, c):
                    hr, hi = c
                    for b in range(8):
                        v = hr * lo_s[0, 8 * sg + b] - hi * lo_s[1, 8 * sg + b]
                        kp_s[8 * j + b] += v[:8] + v[8:]
                    return hr * sr - hi * si, hr * si + hi * sr
                lax.fori_loop(j0, j1, kg, (er * wr - ei * wi, er * wi + ei * wr))
            return c0
        lax.fori_loop(0, N // 16, kchunk, 0)

        def kred8(j, c):
            kd_s[pl.ds(pl.multiple_of(8 * j, 8), 8), :] = jnp.sum(kp_s[pl.ds(8 * j, 8)], axis=1)
            return c
        lax.fori_loop(0, NJ, kred8, 0)
    pl.run_scoped(kgen, pltpu.VMEM((2, 32, 16, D), F32), pltpu.VMEM((8 * NJ, 8, D), F32))

    def kexp(i, c):
        l = i * TM + lax.broadcasted_iota(jnp.int32, (TM, QP), 0)
        q = lax.broadcasted_iota(jnp.int32, (TM, QP), 1)
        st = jnp.where(_l_to_q(l) == q, 1.0, 0.0).astype(BF)
        k_s[pl.ds(i * TM, TM), :] = _dot_sel(st, kd_s[...])
        return c
    lax.fori_loop(0, NT, kexp, 0)

    def ln1(i, c):
        r = pl.ds(i * TM, TM)
        xn_s[r, :] = (_ln(x_ref[r, :].astype(F32))[0]).astype(BF)
        return c
    lax.fori_loop(0, NT, ln1, 0)

    def tr(a, c):
        r = pl.ds(a * C, C)
        u_s[a] = _dot3(fh, fl, xn_s[r, :].astype(F32))
        kf_s[a] = _dot3(fh, fl, k_s[r, :])
        return c
    lax.fori_loop(0, NB, tr, 0)

    def fconv(a, c):
        GR, GI = [], []
        for k0 in range(0, C, 32):
            re = slice(k0, k0 + 32); im = slice(C + k0, C + k0 + 32)

            def inner(dl, cc):
                gr, gi = cc
                b = a - dl
                bm = jnp.maximum(b - 1, 0)
                w = jnp.where(b > 0, 1.0, 0.0) * sgn[:32]
                vr = u_s[b, re, :] - w * u_s[bm, im, :]
                vi = u_s[b, im, :] + w * u_s[bm, re, :]
                kr = kf_s[dl, re, :]; ki = kf_s[dl, im, :]
                return gr + kr * vr - ki * vi, gi + kr * vi + ki * vr
            z0 = jnp.zeros((32, D), F32)
            gr, gi = lax.fori_loop(0, a + 1, inner, (z0, z0))
            GR.append(gr); GI.append(gi)
        y = _r(_dot3(fth, ftl, jnp.concatenate(GR + GI, axis=0)))
        r = pl.ds(a * C, C)
        h_s[r, :] = (_r(x_ref[r, :].astype(F32) + _r(y + _r(xn_s[r, :].astype(F32) * dsk_ref[...].astype(F32))))).astype(BF)
        return c
    lax.fori_loop(0, NB, fconv, 0)

    def gmlp(pre_s, z2n_s, dg_s, acc2_s):
        FH = dg_s.shape[1]

        def f1(i, c):
            r = pl.ds(i * TM, TM)
            hn = _ln(h_s[r, :].astype(F32))[0].astype(BF)
            dx_ref[r, :] = hn
            pre = _dot(hn, win_ref[...]).astype(BF)
            pre_s[r, :] = pre
            z2 = _r(_gelu_and_grad(pre[:, FH:].astype(F32))[0])
            z2n_s[r, :] = _ln(z2)[0].astype(BF)
            return c
        lax.fori_loop(0, NT, f1, 0)

        acc2_s[...] = jnp.zeros(acc2_s.shape, F32)

        def f2(i, c):
            r = pl.ds(i * TM, TM)
            g = _r(_r(_dot(wsp_ref[r, :], z2n_s[...])) + bsp_ref[r, :].astype(F32))
            z1, gp = _gelu_and_grad(pre_s[r, :FH].astype(F32))
            z1 = _r(z1)
            a = (z1 * g).astype(BF)
            out_ref[r, :] = (h_s[r, :].astype(F32) + _r(_dot(a, wout_ref[...]))).astype(BF)
            go = go_ref[r, :]
            acc2_s[...] += _dot_tn(a, go)
            da = _r(_dot_nt(go, wout_ref[...]))
            dg = da * z1
            dbsp_ref[r, :] = jnp.sum(dg, axis=-1, keepdims=True).astype(BF)
            dg_s[r, :] = dg.astype(BF)
            pre_s[r, :FH] = (da * g * gp).astype(BF)
            return c
        lax.fori_loop(0, NT, f2, 0)
        dwout_ref[...] = acc2_s[...].astype(BF)

        def b1(i, c):
            r = pl.ds(i * TM, TM)
            dwsp_ref[r, :] = _dot_nt(dg_s[r, :], z2n_s[...]).astype(BF)
            dz2n = _r(_dot_tn(wsp_ref[:, r], dg_s[...]))
            z, gp = _gelu_and_grad(pre_s[r, FH:].astype(F32))
            xh, sd = _ln(_r(z))
            pre_s[r, FH:] = (_ln_bwd(dz2n, xh, sd) * gp).astype(BF)
            dhn = _dot_nt(pre_s[r, :], win_ref[...])
            hh, hsd = _ln(h_s[r, :].astype(F32))
            h_s[r, :] = (_r(go_ref[r, :].astype(F32) + _ln_bwd(dhn, hh, hsd))).astype(BF)
            return c
        lax.fori_loop(0, NT, b1, 0)

        def b2(i, c):
            cs = pl.ds(pl.multiple_of(i * 512, 512), 512)
            dwin_ref[:, cs] = _dot_tn(dx_ref[...], pre_s[:, cs]).astype(BF)
            return c
        lax.fori_loop(0, 2 * FH // 512, b2, 0)

    FF = win_ref.shape[1]
    pl.run_scoped(gmlp, pltpu.VMEM((L, FF), BF),
                  pltpu.VMEM((L, FF // 2), BF), pltpu.VMEM((L, FF // 2), BF),
                  pltpu.VMEM((FF // 2, D), F32))


    def ssm_bwd(dw_s):
        def tr2(a, c):
            dh = h_s[pl.ds(a * C, C), :].astype(F32)
            dw_s[a] = _dot3(fh, fl, dh)
            return c + jnp.sum(dh * xn_s[pl.ds(a * C, C), :].astype(F32), axis=0, keepdims=True)
        ddsk_ref[...] = lax.fori_loop(0, NB, tr2, jnp.zeros((1, D), F32)).astype(BF)

        def win(a, c):
            ap = jnp.minimum(a + 1, NB - 1)
            w = jnp.where(a + 1 < NB, 1.0, 0.0) * sgn
            nr = dw_s[a, :C, :] + w * dw_s[ap, C:, :]
            ni = dw_s[a, C:, :] - w * dw_s[ap, :C, :]
            dw_s[a, :C, :] = nr
            dw_s[a, C:, :] = ni
            return c
        lax.fori_loop(0, NB, win, 0)

        def bconv(a, c):
            acc = [[], [], [], []]
            for k0 in range(0, C, 16):
                re = slice(k0, k0 + 16); im = slice(C + k0, C + k0 + 16)

                def inner(dl, cc):
                    gr, gi, kr_, ki_ = cc
                    wr_ = dw_s[a + dl, re, :]; wi_ = dw_s[a + dl, im, :]
                    kr = kf_s[dl, re, :]; ki = kf_s[dl, im, :]
                    ur = u_s[dl, re, :]; ui = u_s[dl, im, :]
                    return (gr + kr * wr_ + ki * wi_, gi + kr * wi_ - ki * wr_,
                            kr_ + ur * wr_ + ui * wi_, ki_ + ur * wi_ - ui * wr_)
                z0 = jnp.zeros((16, D), F32)
                for lst, v in zip(acc, lax.fori_loop(0, NB - a, inner, (z0, z0, z0, z0))):
                    lst.append(v)
            r = pl.ds(a * C, C)
            du = _dot3(fth, ftl, jnp.concatenate(acc[0] + acc[1], axis=0))
            k_s[r, :] = _dot3(fth, ftl, jnp.concatenate(acc[2] + acc[3], axis=0))
            dh = h_s[r, :].astype(F32)
            dxn = du + dh * dsk_ref[...].astype(F32)
            xh, sd = _ln(x_ref[r, :].astype(F32))
            dx_ref[r, :] = (dh + _ln_bwd(dxn, xh, sd)).astype(BF)
            return c
        lax.fori_loop(0, NB, bconv, 0)

    pl.run_scoped(ssm_bwd, pltpu.VMEM((NB, 2 * C, D), F32))

    kd_s[...] = jnp.zeros(kd_s.shape, F32)

    def kred(i, c):
        q = lax.broadcasted_iota(jnp.int32, (QP, TM), 0)
        l = i * TM + lax.broadcasted_iota(jnp.int32, (QP, TM), 1)
        kd_s[...] += _dot_sel(jnp.where(_l_to_q(l) == q, 1.0, 0.0).astype(BF),
                              k_s[pl.ds(i * TM, TM), :])
        return c
    lax.fori_loop(0, NT, kred, 0)
    def pgrad(lo_s):
        def chunk(nc, c0):
            rn = pl.ds(pl.multiple_of(nc * 16, 16), 16)
            fill_lo(lo_s, rn)
            z = jnp.zeros((16, D), F32)
            g = (z, z, z, z)
            for sg, (j0, j1) in enumerate(SEG):
                sr, si = cexp(float(8 << sg), rn)

                def pg(j, c):
                    hr, hi, g1r, g1i, g2r, g2i = c
                    t1r = t1i = t2r = t2i = z
                    for b in range(8):
                        d1 = kd_s[pl.ds(8 * j + b, 1), :]
                        d2 = d1 * float(b << sg)
                        lr = lo_s[0, 8 * sg + b]; li = lo_s[1, 8 * sg + b]
                        t1r = t1r + d1 * lr; t1i = t1i + d1 * li
                        t2r = t2r + d2 * lr; t2i = t2i + d2 * li
                    rh = _q_to_r(8 * j).astype(F32)
                    t2r = t2r + rh * t1r; t2i = t2i + rh * t1i
                    return (hr * sr - hi * si, hr * si + hi * sr,
                            g1r + hr * t1r - hi * t1i, g1i + hr * t1i + hi * t1r,
                            g2r + hr * t2r - hi * t2i, g2i + hr * t2i + hi * t2r)
                g = lax.fori_loop(j0, j1, pg, cexp(float((0, 256, 512, 1024)[sg]), rn) + tuple(g))[2:]
            dare_ref[rn, :], daim_ref[rn, :], dbre_ref[rn, :], dbim_ref[rn, :] = g
            return c0
        lax.fori_loop(0, N // 16, chunk, 0)
        g = (dare_ref[...], daim_ref[...], dbre_ref[...], dbim_ref[...])
        g1r, g1i, g2r, g2i = g
        wr, wi = wmat()
        br = bre_ref[...] * dt; bi = bim_ref[...] * dt
        cr = cre_ref[...]; ci = cim_ref[...]
        gwr, gwi = g1r, -g1i
        glr = wr * g2r - wi * g2i
        gli = -(wr * g2i + wi * g2r)
        gbr = gwr * cr + gwi * ci; gbi = gwi * cr - gwr * ci
        dcre_ref[...] = gwr * br + gwi * bi; dcim_ref[...] = gwi * br - gwr * bi
        dbre_ref[...] = gbr * dt; dbim_ref[...] = gbi * dt
        dare_ref[...] = glr * dt; daim_ref[...] = gli * dt
        dldt_ref[...] = jnp.sum(gbr * br + gbi * bi + dt * (glr * are_ref[...] + gli * aim_ref[...]),
                                axis=0, keepdims=True).astype(BF)
    pl.run_scoped(pgrad, pltpu.VMEM((2, 32, 16, D), F32))


@jax.jit
def pallas_sequential_preLN__ssm_conv_s4__mixer_gmlp__prompt_kernel(
    A_u, A_A_re, A_A_im, A_B_re, A_B_im, A_C_re, A_C_im, A_log_dt, A_Dskip,
    B_x, B_w_in, B_w_sp, B_b_sp, B_w_out, grad_out,
):
    _, L, D = A_u.shape
    N = A_A_re.shape[1]
    F = B_w_in.shape[1]
    FH = F // 2
    S = jax.ShapeDtypeStruct
    nd = S((N, D), F32)
    outs = pl.pallas_call(
        _kernel,
        out_shape=(S((L, D), BF), S((L, D), BF), nd, nd, nd, nd, nd, nd, S((1, D), BF), S((1, D), BF),
                   S((D, F), BF), S((L, L), BF), S((L, 1), BF), S((FH, D), BF)),
        scratch_shapes=[
            pltpu.VMEM((L, D), BF), pltpu.VMEM((L, D), BF),
            pltpu.VMEM((L, D), F32), pltpu.VMEM((QP, D), F32),
            pltpu.VMEM((L // C, 2 * C, D), F32), pltpu.VMEM((L // C, 2 * C, D), F32),
        ],
        compiler_params=pltpu.CompilerParams(vmem_limit_bytes=127 * 1024 * 1024),
    )(A_u[0], A_A_re.T.astype(F32), A_A_im.T.astype(F32), A_B_re.T.astype(F32), A_B_im.T.astype(F32), A_C_re.T.astype(F32), A_C_im.T.astype(F32),
      A_log_dt.reshape(1, D), A_Dskip.reshape(1, D), B_w_in, B_w_sp, B_b_sp.reshape(L, 1),
      B_w_out, grad_out[0])
    o, dx, a1, a2, b1, b2, c1, c2, dl, dd, dwi, dws, dbs, dwo = outs
    return (o[None], dx[None], a1.T.astype(BF), a2.T.astype(BF), b1.T.astype(BF), b2.T.astype(BF), c1.T.astype(BF), c2.T.astype(BF), dl.reshape(D), dd.reshape(D),
            dwi, dws, dbs.reshape(L), dwo)
```

```python
import math
import jax
import jax.numpy as jnp
from jax import lax
import jax.experimental.pallas as pl
import jax.experimental.pallas.tpu as pltpu

BF = jnp.bfloat16
F32 = jnp.float32
EPS = 1e-5
C = 128
TM = 128
QP = 768


def _dot(a, b):
    return jnp.dot(a, b, preferred_element_type=F32)


def _dot_tn(a, b):
    return lax.dot_general(a, b, (((0,), (0,)), ((), ())), preferred_element_type=F32)


def _dot_nt(a, b):
    return lax.dot_general(a, b, (((1,), (1,)), ((), ())), preferred_element_type=F32)


def _split(x):
    hi = x.astype(BF)
    return hi, (x - hi.astype(F32)).astype(BF)


def _dot3(fh, fl, x):
    xh, xl = _split(x)
    return _dot(fh, xh) + _dot(fh, xl) + _dot(fl, xh)


def _dot_sel(s, x):
    xh, xl = _split(x)
    xl2 = (x - xh.astype(F32) - xl.astype(F32)).astype(BF)
    return _dot(s, xh) + _dot(s, xl) + _dot(s, xl2)


def _r(x):
    return x.astype(BF).astype(F32)


def _ln(x):
    m = _r(jnp.mean(x, axis=-1, keepdims=True))
    v = _r(jnp.mean(jnp.square(x - jnp.mean(x, axis=-1, keepdims=True)), axis=-1, keepdims=True))
    sd = _r(jnp.sqrt(_r(v + EPS)))
    return _r(_r(x - m) / sd), sd


def _ln_bwd(dy, xh, sd):
    return (dy - jnp.mean(dy, axis=-1, keepdims=True)
            - xh * jnp.mean(dy * xh, axis=-1, keepdims=True)) / sd


_GC = math.sqrt(2.0 / math.pi)


def _gelu_and_grad(x):
    u = _GC * (x + 0.044715 * x * x * x)
    t = jnp.tanh(u)
    g = 0.5 * x * (1.0 + t)
    dg = 0.5 * (1.0 + t) + 0.5 * x * (1.0 - t * t) * _GC * (1.0 + 3 * 0.044715 * x * x)
    return g, dg


def _q_to_r(q):
    return jnp.where(q < 256, q, jnp.where(q < 384, 256 + 2 * (q - 256),
                     jnp.where(q < 512, 512 + 4 * (q - 384), 1024 + 8 * (q - 512))))


def _l_to_q(l):
    r = l.astype(F32).astype(BF).astype(F32).astype(jnp.int32)
    return jnp.where(r < 256, r, jnp.where(r < 512, 256 + (r - 256) // 2,
                     jnp.where(r < 1024, 384 + (r - 512) // 4, 512 + (r - 1024) // 8)))


def _seg(j):
    return 0 if j < 32 else (1 if j < 48 else (2 if j < 64 else 3))


def _kernel(x_ref, are_ref, aim_ref, bre_ref, bim_ref, cre_ref, cim_ref, ldt_ref, dsk_ref,
            win_ref, wsp_ref, bsp_ref, wout_ref, go_ref,
            out_ref, dx_ref, dare_ref, daim_ref, dbre_ref, dbim_ref, dcre_ref, dcim_ref,
            dldt_ref, ddsk_ref, dwin_ref, dwsp_ref, dbsp_ref, dwout_ref,
            xn_s, h_s, k_s, kd_s, u_s, kf_s):
    L, D = x_ref.shape
    N = are_ref.shape[0]
    NB = L // C
    NT = L // TM
    NJ = 81

    def dft(shape, kax):
        k = lax.broadcasted_iota(jnp.int32, shape, kax)
        t = lax.broadcasted_iota(jnp.int32, shape, 1 - kax)
        ang = (((2 * (k % C) + 1) * t) % (4 * C)).astype(F32) * (math.pi / (2 * C))
        return jnp.where(k < C, jnp.cos(ang), -jnp.sin(ang))
    fh, fl = _split(dft((2 * C, C), 0))
    fth, ftl = _split(dft((C, 2 * C), 1) * (1.0 / C))
    sgn = (1 - 2 * (lax.broadcasted_iota(jnp.int32, (C, 1), 0) % 2)).astype(F32)

    dt = _r(jnp.exp(ldt_ref[...].astype(F32)))

    SEG = ((0, 32), (32, 48), (48, 64), (64, 81))

    def cexp(r, rn=slice(None)):
        e = jnp.exp(are_ref[rn, :] * dt * r)
        th = aim_ref[rn, :] * dt * r
        return e * jnp.cos(th), e * jnp.sin(th)

    def wmat(rn=slice(None)):
        br = bre_ref[rn, :] * dt; bi = bim_ref[rn, :] * dt
        cr = cre_ref[rn, :]; ci = cim_ref[rn, :]
        return cr * br - ci * bi, cr * bi + ci * br

    def fill_lo(lo_s, rn=slice(None)):
        er, ei = cexp(1.0, rn)
        for sg in range(4):
            pr = jnp.ones_like(er); pi_ = jnp.zeros_like(er)
            for b in range(8):
                lo_s[0, 8 * sg + b] = pr; lo_s[1, 8 * sg + b] = pi_
                pr, pi_ = pr * er - pi_ * ei, pr * ei + pi_ * er
            er, ei = er * er - ei * ei, 2.0 * er * ei

    kd_s[...] = jnp.zeros(kd_s.shape, F32)

    def kgen(lo_s, kp_s):
        kp_s[...] = jnp.zeros(kp_s.shape, F32)

        def kchunk(nc, c0):
            rn = pl.ds(pl.multiple_of(nc * 16, 16), 16)
            fill_lo(lo_s, rn)
            wr, wi = wmat(rn)
            for sg, (j0, j1) in enumerate(SEG):
                er, ei = cexp(float((0, 256, 512, 1024)[sg]), rn)
                sr, si = cexp(float(8 << sg), rn)

                def kg(j, c):
                    hr, hi = c
                    for b in range(8):
                        v = hr * lo_s[0, 8 * sg + b] - hi * lo_s[1, 8 * sg + b]
                        kp_s[8 * j + b] += v[:8] + v[8:]
                    return hr * sr - hi * si, hr * si + hi * sr
                lax.fori_loop(j0, j1, kg, (er * wr - ei * wi, er * wi + ei * wr))
            return c0
        lax.fori_loop(0, N // 16, kchunk, 0)

        def kred8(j, c):
            kd_s[pl.ds(pl.multiple_of(8 * j, 8), 8), :] = jnp.sum(kp_s[pl.ds(8 * j, 8)], axis=1)
            return c
        lax.fori_loop(0, NJ, kred8, 0)
    pl.run_scoped(kgen, pltpu.VMEM((2, 32, 16, D), F32), pltpu.VMEM((8 * NJ, 8, D), F32))

    def qwin(i):
        q0 = jnp.minimum((_l_to_q(i * C) // 128) * 128, QP - 256)
        return pl.multiple_of(q0, 128)

    def kexp(i, c):
        q0 = qwin(i)
        l = i * C + lax.broadcasted_iota(jnp.int32, (C, 256), 0)
        q = q0 + lax.broadcasted_iota(jnp.int32, (C, 256), 1)
        st = jnp.where(_l_to_q(l) == q, 1.0, 0.0).astype(BF)
        k_s[pl.ds(i * C, C), :] = _dot_sel(st, kd_s[pl.ds(q0, 256), :])
        return c
    lax.fori_loop(0, NB, kexp, 0)

    def ln1(i, c):
        r = pl.ds(i * TM, TM)
        xn_s[r, :] = (_ln(x_ref[r, :].astype(F32))[0]).astype(BF)
        return c
    lax.fori_loop(0, NT, ln1, 0)

    def tr(a, c):
        r = pl.ds(a * C, C)
        u_s[a] = _dot3(fh, fl, xn_s[r, :].astype(F32))
        kf_s[a] = _dot3(fh, fl, k_s[r, :])
        return c
    lax.fori_loop(0, NB, tr, 0)

    def fconv(a, c):
        GR, GI = [], []
        for k0 in range(0, C, 32):
            re = slice(k0, k0 + 32); im = slice(C + k0, C + k0 + 32)

            def inner(dl, cc):
                gr, gi = cc
                b = a - dl
                bm = jnp.maximum(b - 1, 0)
                w = jnp.where(b > 0, 1.0, 0.0) * sgn[:32]
                vr = u_s[b, re, :] - w * u_s[bm, im, :]
                vi = u_s[b, im, :] + w * u_s[bm, re, :]
                kr = kf_s[dl, re, :]; ki = kf_s[dl, im, :]
                return gr + kr * vr - ki * vi, gi + kr * vi + ki * vr
            z0 = jnp.zeros((32, D), F32)
            gr, gi = lax.fori_loop(0, a + 1, inner, (z0, z0))
            GR.append(gr); GI.append(gi)
        y = _r(_dot3(fth, ftl, jnp.concatenate(GR + GI, axis=0)))
        r = pl.ds(a * C, C)
        h_s[r, :] = (_r(x_ref[r, :].astype(F32) + _r(y + _r(xn_s[r, :].astype(F32) * dsk_ref[...].astype(F32))))).astype(BF)
        return c
    lax.fori_loop(0, NB, fconv, 0)

    def gmlp(pre_s, z2n_s, dg_s, acc2_s):
        FH = dg_s.shape[1]

        def f1(i, c):
            r = pl.ds(i * TM, TM)
            hn = _ln(h_s[r, :].astype(F32))[0].astype(BF)
            dx_ref[r, :] = hn
            pre = _dot(hn, win_ref[...]).astype(BF)
            pre_s[r, :] = pre
            z2 = _r(_gelu_and_grad(pre[:, FH:].astype(F32))[0])
            z2n_s[r, :] = _ln(z2)[0].astype(BF)
            return c
        lax.fori_loop(0, NT, f1, 0)

        acc2_s[...] = jnp.zeros(acc2_s.shape, F32)

        def f2(i, c):
            r = pl.ds(i * TM, TM)
            g = _r(_r(_dot(wsp_ref[r, :], z2n_s[...])) + bsp_ref[r, :].astype(F32))
            z1, gp = _gelu_and_grad(pre_s[r, :FH].astype(F32))
            z1 = _r(z1)
            a = (z1 * g).astype(BF)
            out_ref[r, :] = (h_s[r, :].astype(F32) + _r(_dot(a, wout_ref[...]))).astype(BF)
            go = go_ref[r, :]
            acc2_s[...] += _dot_tn(a, go)
            da = _r(_dot_nt(go, wout_ref[...]))
            dg = da * z1
            dbsp_ref[r, :] = jnp.sum(dg, axis=-1, keepdims=True).astype(BF)
            dg_s[r, :] = dg.astype(BF)
            pre_s[r, :FH] = (da * g * gp).astype(BF)
            return c
        lax.fori_loop(0, NT, f2, 0)
        dwout_ref[...] = acc2_s[...].astype(BF)

        def b1(i, c):
            r = pl.ds(i * TM, TM)
            dwsp_ref[r, :] = _dot_nt(dg_s[r, :], z2n_s[...]).astype(BF)
            dz2n = _r(_dot_tn(wsp_ref[:, r], dg_s[...]))
            z, gp = _gelu_and_grad(pre_s[r, FH:].astype(F32))
            xh, sd = _ln(_r(z))
            pre_s[r, FH:] = (_ln_bwd(dz2n, xh, sd) * gp).astype(BF)
            dhn = _dot_nt(pre_s[r, :], win_ref[...])
            hh, hsd = _ln(h_s[r, :].astype(F32))
            h_s[r, :] = (_r(go_ref[r, :].astype(F32) + _ln_bwd(dhn, hh, hsd))).astype(BF)
            return c
        lax.fori_loop(0, NT, b1, 0)

        def b2(i, c):
            cs = pl.ds(pl.multiple_of(i * 512, 512), 512)
            dwin_ref[:, cs] = _dot_tn(dx_ref[...], pre_s[:, cs]).astype(BF)
            return c
        lax.fori_loop(0, 2 * FH // 512, b2, 0)

    FF = win_ref.shape[1]
    pl.run_scoped(gmlp, pltpu.VMEM((L, FF), BF),
                  pltpu.VMEM((L, FF // 2), BF), pltpu.VMEM((L, FF // 2), BF),
                  pltpu.VMEM((FF // 2, D), F32))


    def ssm_bwd(dw_s):
        def tr2(a, c):
            dh = h_s[pl.ds(a * C, C), :].astype(F32)
            dw_s[a] = _dot3(fh, fl, dh)
            return c + jnp.sum(dh * xn_s[pl.ds(a * C, C), :].astype(F32), axis=0, keepdims=True)
        ddsk_ref[...] = lax.fori_loop(0, NB, tr2, jnp.zeros((1, D), F32)).astype(BF)

        def win(a, c):
            ap = jnp.minimum(a + 1, NB - 1)
            w = jnp.where(a + 1 < NB, 1.0, 0.0) * sgn
            nr = dw_s[a, :C, :] + w * dw_s[ap, C:, :]
            ni = dw_s[a, C:, :] - w * dw_s[ap, :C, :]
            dw_s[a, :C, :] = nr
            dw_s[a, C:, :] = ni
            return c
        lax.fori_loop(0, NB, win, 0)

        def bconv(a, c):
            acc = [[], [], [], []]
            for k0 in range(0, C, 16):
                re = slice(k0, k0 + 16); im = slice(C + k0, C + k0 + 16)

                def inner(dl, cc):
                    gr, gi, kr_, ki_ = cc
                    wr_ = dw_s[a + dl, re, :]; wi_ = dw_s[a + dl, im, :]
                    kr = kf_s[dl, re, :]; ki = kf_s[dl, im, :]
                    ur = u_s[dl, re, :]; ui = u_s[dl, im, :]
                    return (gr + kr * wr_ + ki * wi_, gi + kr * wi_ - ki * wr_,
                            kr_ + ur * wr_ + ui * wi_, ki_ + ur * wi_ - ui * wr_)
                z0 = jnp.zeros((16, D), F32)
                for lst, v in zip(acc, lax.fori_loop(0, NB - a, inner, (z0, z0, z0, z0))):
                    lst.append(v)
            r = pl.ds(a * C, C)
            du = _dot3(fth, ftl, jnp.concatenate(acc[0] + acc[1], axis=0))
            k_s[r, :] = _dot3(fth, ftl, jnp.concatenate(acc[2] + acc[3], axis=0))
            dh = h_s[r, :].astype(F32)
            dxn = du + dh * dsk_ref[...].astype(F32)
            xh, sd = _ln(x_ref[r, :].astype(F32))
            dx_ref[r, :] = (dh + _ln_bwd(dxn, xh, sd)).astype(BF)
            return c
        lax.fori_loop(0, NB, bconv, 0)

    pl.run_scoped(ssm_bwd, pltpu.VMEM((NB, 2 * C, D), F32))

    kd_s[...] = jnp.zeros(kd_s.shape, F32)

    def kred(i, c):
        q0 = qwin(i)
        q = q0 + lax.broadcasted_iota(jnp.int32, (256, C), 0)
        l = i * C + lax.broadcasted_iota(jnp.int32, (256, C), 1)
        kd_s[pl.ds(q0, 256), :] += _dot_sel(jnp.where(_l_to_q(l) == q, 1.0, 0.0).astype(BF),
                                            k_s[pl.ds(i * C, C), :])
        return c
    lax.fori_loop(0, NB, kred, 0)

    def pgrad(lo_s, st_s):
        outs = (dare_ref, daim_ref, dbre_ref, dbim_ref)

        def chunk(nc, c0):
            rn = pl.ds(pl.multiple_of(nc * 16, 16), 16)
            fill_lo(lo_s, rn)
            z = jnp.zeros((16, D), F32)
            for o in outs:
                o[rn, :] = z
            for sg, (j0, j1) in enumerate(SEG):
                st_s[0], st_s[1] = cexp(float((0, 256, 512, 1024)[sg]), rn)
                st_s[2], st_s[3] = cexp(float(8 << sg), rn)

                def pg(j, c):
                    t1r = t1i = t2r = t2i = z
                    for b in range(8):
                        d1 = kd_s[pl.ds(8 * j + b, 1), :]
                        d2 = d1 * float(b << sg)
                        lr = lo_s[0, 8 * sg + b]; li = lo_s[1, 8 * sg + b]
                        t1r = t1r + d1 * lr; t1i = t1i + d1 * li
                        t2r = t2r + d2 * lr; t2i = t2i + d2 * li
                    rh = _q_to_r(8 * j).astype(F32)
                    t2r = t2r + rh * t1r; t2i = t2i + rh * t1i
                    hr = st_s[0]; hi = st_s[1]
                    dare_ref[rn, :] += hr * t1r - hi * t1i
                    daim_ref[rn, :] += hr * t1i + hi * t1r
                    dbre_ref[rn, :] += hr * t2r - hi * t2i
                    dbim_ref[rn, :] += hr * t2i + hi * t2r
                    sr = st_s[2]; si = st_s[3]
                    st_s[0] = hr * sr - hi * si
                    st_s[1] = hr * si + hi * sr
                    return c
                lax.fori_loop(j0, j1, pg, 0)
            return c0
        lax.fori_loop(0, N // 16, chunk, 0)
        g = (dare_ref[...], daim_ref[...], dbre_ref[...], dbim_ref[...])
        g1r, g1i, g2r, g2i = g
        wr, wi = wmat()
        br = bre_ref[...] * dt; bi = bim_ref[...] * dt
        cr = cre_ref[...]; ci = cim_ref[...]
        gwr, gwi = g1r, -g1i
        glr = wr * g2r - wi * g2i
        gli = -(wr * g2i + wi * g2r)
        gbr = gwr * cr + gwi * ci; gbi = gwi * cr - gwr * ci
        dcre_ref[...] = gwr * br + gwi * bi; dcim_ref[...] = gwi * br - gwr * bi
        dbre_ref[...] = gbr * dt; dbim_ref[...] = gbi * dt
        dare_ref[...] = glr * dt; daim_ref[...] = gli * dt
        dldt_ref[...] = jnp.sum(gbr * br + gbi * bi + dt * (glr * are_ref[...] + gli * aim_ref[...]),
                                axis=0, keepdims=True).astype(BF)
    pl.run_scoped(pgrad, pltpu.VMEM((2, 32, 16, D), F32), pltpu.VMEM((4, 16, D), F32))


@jax.jit
def pallas_sequential_preLN__ssm_conv_s4__mixer_gmlp__prompt_kernel(
    A_u, A_A_re, A_A_im, A_B_re, A_B_im, A_C_re, A_C_im, A_log_dt, A_Dskip,
    B_x, B_w_in, B_w_sp, B_b_sp, B_w_out, grad_out,
):
    _, L, D = A_u.shape
    N = A_A_re.shape[1]
    F = B_w_in.shape[1]
    FH = F // 2
    S = jax.ShapeDtypeStruct
    nd = S((N, D), F32)
    outs = pl.pallas_call(
        _kernel,
        out_shape=(S((L, D), BF), S((L, D), BF), nd, nd, nd, nd, nd, nd, S((1, D), BF), S((1, D), BF),
                   S((D, F), BF), S((L, L), BF), S((L, 1), BF), S((FH, D), BF)),
        scratch_shapes=[
            pltpu.VMEM((L, D), BF), pltpu.VMEM((L, D), BF),
            pltpu.VMEM((L, D), F32), pltpu.VMEM((QP, D), F32),
            pltpu.VMEM((L // C, 2 * C, D), F32), pltpu.VMEM((L // C, 2 * C, D), F32),
        ],
        compiler_params=pltpu.CompilerParams(vmem_limit_bytes=127 * 1024 * 1024),
    )(A_u[0], A_A_re.T.astype(F32), A_A_im.T.astype(F32), A_B_re.T.astype(F32), A_B_im.T.astype(F32), A_C_re.T.astype(F32), A_C_im.T.astype(F32),
      A_log_dt.reshape(1, D), A_Dskip.reshape(1, D), B_w_in, B_w_sp, B_b_sp.reshape(L, 1),
      B_w_out, grad_out[0])
    o, dx, a1, a2, b1, b2, c1, c2, dl, dd, dwi, dws, dbs, dwo = outs
    return (o[None], dx[None], a1.T.astype(BF), a2.T.astype(BF), b1.T.astype(BF), b2.T.astype(BF), c1.T.astype(BF), c2.T.astype(BF), dl.reshape(D), dd.reshape(D),
            dwi, dws, dbs.reshape(L), dwo)
```

```python
import math
import jax
import jax.numpy as jnp
from jax import lax
import jax.experimental.pallas as pl
import jax.experimental.pallas.tpu as pltpu

BF = jnp.bfloat16
F32 = jnp.float32
EPS = 1e-5
C = 128
TM = 128
QP = 768


def _dot(a, b):
    return jnp.dot(a, b, preferred_element_type=F32)


def _dot_tn(a, b):
    return lax.dot_general(a, b, (((0,), (0,)), ((), ())), preferred_element_type=F32)


def _dot_nt(a, b):
    return lax.dot_general(a, b, (((1,), (1,)), ((), ())), preferred_element_type=F32)


def _split(x):
    hi = x.astype(BF)
    return hi, (x - hi.astype(F32)).astype(BF)


def _dot3(fh, fl, x):
    xh, xl = _split(x)
    return _dot(fh, xh) + _dot(fh, xl) + _dot(fl, xh)


def _dot_sel(s, x):
    xh, xl = _split(x)
    xl2 = (x - xh.astype(F32) - xl.astype(F32)).astype(BF)
    return _dot(s, xh) + _dot(s, xl) + _dot(s, xl2)


def _r(x):
    return x.astype(BF).astype(F32)


def _ln(x):
    m = _r(jnp.mean(x, axis=-1, keepdims=True))
    v = _r(jnp.mean(jnp.square(x - jnp.mean(x, axis=-1, keepdims=True)), axis=-1, keepdims=True))
    sd = _r(jnp.sqrt(_r(v + EPS)))
    return _r(_r(x - m) / sd), sd


def _ln_bwd(dy, xh, sd):
    return (dy - jnp.mean(dy, axis=-1, keepdims=True)
            - xh * jnp.mean(dy * xh, axis=-1, keepdims=True)) / sd


_GC = math.sqrt(2.0 / math.pi)


def _gelu_and_grad(x):
    u = _GC * (x + 0.044715 * x * x * x)
    t = jnp.tanh(u)
    g = 0.5 * x * (1.0 + t)
    dg = 0.5 * (1.0 + t) + 0.5 * x * (1.0 - t * t) * _GC * (1.0 + 3 * 0.044715 * x * x)
    return g, dg


def _q_to_r(q):
    return jnp.where(q < 256, q, jnp.where(q < 384, 256 + 2 * (q - 256),
                     jnp.where(q < 512, 512 + 4 * (q - 384), 1024 + 8 * (q - 512))))


def _l_to_q(l):
    r = l.astype(F32).astype(BF).astype(F32).astype(jnp.int32)
    return jnp.where(r < 256, r, jnp.where(r < 512, 256 + (r - 256) // 2,
                     jnp.where(r < 1024, 384 + (r - 512) // 4, 512 + (r - 1024) // 8)))


def _seg(j):
    return 0 if j < 32 else (1 if j < 48 else (2 if j < 64 else 3))


def _kernel(x_ref, i0, i1, i2, i3, i4, i5, ldt_ref, dsk_ref,
            win_h, wsp_h, bsp_ref, wout_h, go_h,
            out_ref, dx_ref, o0, o1, o2, o3, o4, o5,
            dldt_ref, ddsk_ref, dwin_ref, dwsp_ref, dbsp_ref, dwout_ref,
            xn_s, h_s, k_s, kd_s, u_s, kf_s, win_ref, wsp_ref, wout_ref, go_ref, isem, pin_s, pout_s):
    for k_, r_ in enumerate((i0, i1, i2, i3, i4, i5)):
        pin_s[k_] = r_[...].astype(F32).T
    are_ref, aim_ref, bre_ref, bim_ref, cre_ref, cim_ref = [pin_s.at[k_] for k_ in range(6)]
    dare_ref, daim_ref, dbre_ref, dbim_ref, dcre_ref, dcim_ref = [pout_s.at[k_] for k_ in range(6)]
    in_cp = [pltpu.make_async_copy(a_, b_, isem.at[i_]) for i_, (a_, b_) in enumerate(
        ((win_h, win_ref), (wsp_h, wsp_ref), (wout_h, wout_ref), (go_h, go_ref)))]
    for cp in in_cp:
        cp.start()
    L, D = x_ref.shape
    N = are_ref.shape[0]
    NB = L // C
    NT = L // TM
    NJ = 81

    def dft(shape, kax):
        k = lax.broadcasted_iota(jnp.int32, shape, kax)
        t = lax.broadcasted_iota(jnp.int32, shape, 1 - kax)
        ang = (((2 * (k % C) + 1) * t) % (4 * C)).astype(F32) * (math.pi / (2 * C))
        return jnp.where(k < C, jnp.cos(ang), -jnp.sin(ang))
    fh, fl = _split(dft((2 * C, C), 0))
    fth, ftl = _split(dft((C, 2 * C), 1) * (1.0 / C))
    sgn = (1 - 2 * (lax.broadcasted_iota(jnp.int32, (C, 1), 0) % 2)).astype(F32)

    dt = _r(jnp.exp(ldt_ref[...].astype(F32)))

    SEG = ((0, 32), (32, 48), (48, 64), (64, 81))

    def cexp(r, rn=slice(None)):
        e = jnp.exp(are_ref[rn, :] * dt * r)
        th = aim_ref[rn, :] * dt * r
        return e * jnp.cos(th), e * jnp.sin(th)

    def wmat(rn=slice(None)):
        br = bre_ref[rn, :] * dt; bi = bim_ref[rn, :] * dt
        cr = cre_ref[rn, :]; ci = cim_ref[rn, :]
        return cr * br - ci * bi, cr * bi + ci * br

    def fill_lo(lo_s, rn=slice(None)):
        er, ei = cexp(1.0, rn)
        for sg in range(4):
            pr = jnp.ones_like(er); pi_ = jnp.zeros_like(er)
            for b in range(8):
                lo_s[0, 8 * sg + b] = pr; lo_s[1, 8 * sg + b] = pi_
                pr, pi_ = pr * er - pi_ * ei, pr * ei + pi_ * er
            er, ei = er * er - ei * ei, 2.0 * er * ei

    kd_s[...] = jnp.zeros(kd_s.shape, F32)

    def kgen(lo_s, kp_s):
        kp_s[...] = jnp.zeros(kp_s.shape, F32)

        def kchunk(nc, c0):
            rn = pl.ds(pl.multiple_of(nc * 16, 16), 16)
            fill_lo(lo_s, rn)
            wr, wi = wmat(rn)
            for sg, (j0, j1) in enumerate(SEG):
                er, ei = cexp(float((0, 256, 512, 1024)[sg]), rn)
                sr, si = cexp(float(8 << sg), rn)

                def kg(j, c):
                    hr, hi = c
                    for b in range(8):
                        v = hr * lo_s[0, 8 * sg + b] - hi * lo_s[1, 8 * sg + b]
                        kp_s[8 * j + b] += v[:8] + v[8:]
                    return hr * sr - hi * si, hr * si + hi * sr
                lax.fori_loop(j0, j1, kg, (er * wr - ei * wi, er * wi + ei * wr))
            return c0
        lax.fori_loop(0, N // 16, kchunk, 0)

        def kred8(j, c):
            kd_s[pl.ds(pl.multiple_of(8 * j, 8), 8), :] = jnp.sum(kp_s[pl.ds(8 * j, 8)], axis=1)
            return c
        lax.fori_loop(0, NJ, kred8, 0)
    pl.run_scoped(kgen, pltpu.VMEM((2, 32, 16, D), F32), pltpu.VMEM((8 * NJ, 8, D), F32))

    def qwin(i):
        q0 = jnp.minimum((_l_to_q(i * C) // 128) * 128, QP - 256)
        return pl.multiple_of(q0, 128)

    def kexp(i, c):
        q0 = qwin(i)
        l = i * C + lax.broadcasted_iota(jnp.int32, (C, 256), 0)
        q = q0 + lax.broadcasted_iota(jnp.int32, (C, 256), 1)
        st = jnp.where(_l_to_q(l) == q, 1.0, 0.0).astype(BF)
        k_s[pl.ds(i * C, C), :] = _dot_sel(st, kd_s[pl.ds(q0, 256), :])
        return c
    lax.fori_loop(0, NB, kexp, 0)

    def ln1(i, c):
        r = pl.ds(i * TM, TM)
        xn_s[r, :] = (_ln(x_ref[r, :].astype(F32))[0]).astype(BF)
        return c
    lax.fori_loop(0, NT, ln1, 0)

    def tr(a, c):
        r = pl.ds(a * C, C)
        u_s[a] = _dot3(fh, fl, xn_s[r, :].astype(F32))
        kf_s[a] = _dot3(fh, fl, k_s[r, :])
        return c
    lax.fori_loop(0, NB, tr, 0)

    def fconv(a, c):
        GR, GI = [], []
        for k0 in range(0, C, 32):
            re = slice(k0, k0 + 32); im = slice(C + k0, C + k0 + 32)

            def inner(dl, cc):
                gr, gi = cc
                b = a - dl
                bm = jnp.maximum(b - 1, 0)
                w = jnp.where(b > 0, 1.0, 0.0) * sgn[:32]
                vr = u_s[b, re, :] - w * u_s[bm, im, :]
                vi = u_s[b, im, :] + w * u_s[bm, re, :]
                kr = kf_s[dl, re, :]; ki = kf_s[dl, im, :]
                return gr + kr * vr - ki * vi, gi + kr * vi + ki * vr
            z0 = jnp.zeros((32, D), F32)
            gr, gi = lax.fori_loop(0, a + 1, inner, (z0, z0))
            GR.append(gr); GI.append(gi)
        y = _r(_dot3(fth, ftl, jnp.concatenate(GR + GI, axis=0)))
        r = pl.ds(a * C, C)
        h_s[r, :] = (_r(x_ref[r, :].astype(F32) + _r(y + _r(xn_s[r, :].astype(F32) * dsk_ref[...].astype(F32))))).astype(BF)
        return c
    lax.fori_loop(0, NB, fconv, 0)

    def gmlp(pre_s, z2n_s, dg_s, acc2_s, buf1, buf2, sem1, sem2):
        for cp in in_cp:
            cp.wait()
        FH = dg_s.shape[1]

        def f1(i, c):
            r = pl.ds(i * TM, TM)
            hn = _ln(h_s[r, :].astype(F32))[0].astype(BF)
            dx_ref[r, :] = hn
            pre = _dot(hn, win_ref[...]).astype(BF)
            pre_s[r, :] = pre
            z2 = _r(_gelu_and_grad(pre[:, FH:].astype(F32))[0])
            z2n_s[r, :] = _ln(z2)[0].astype(BF)
            return c
        lax.fori_loop(0, NT, f1, 0)

        acc2_s[...] = jnp.zeros(acc2_s.shape, F32)

        def f2(i, c):
            r = pl.ds(i * TM, TM)
            g = _r(_r(_dot(wsp_ref[r, :], z2n_s[...])) + bsp_ref[r, :].astype(F32))
            z1, gp = _gelu_and_grad(pre_s[r, :FH].astype(F32))
            z1 = _r(z1)
            a = (z1 * g).astype(BF)
            out_ref[r, :] = (h_s[r, :].astype(F32) + _r(_dot(a, wout_ref[...]))).astype(BF)
            go = go_ref[r, :]
            acc2_s[...] += _dot_tn(a, go)
            da = _r(_dot_nt(go, wout_ref[...]))
            dg = da * z1
            dbsp_ref[r, :] = jnp.sum(dg, axis=-1, keepdims=True).astype(BF)
            dg_s[r, :] = dg.astype(BF)
            pre_s[r, :FH] = (da * g * gp).astype(BF)
            return c
        lax.fori_loop(0, NT, f2, 0)
        dwout_ref[...] = acc2_s[...].astype(BF)

        def cp1(i):
            return pltpu.make_async_copy(buf1.at[i % 2], dwsp_ref.at[pl.ds(i * TM, TM), :],
                                         sem1.at[i % 2])

        def cp2(i):
            return pltpu.make_async_copy(buf2.at[i % 2], dwin_ref.at[:, pl.ds(i * 512, 512)],
                                         sem2.at[i % 2])

        def b1(i, c):
            r = pl.ds(i * TM, TM)
            sl = i % 2

            @pl.when(i >= 2)
            def _():
                cp1(i - 2).wait()
            buf1[sl] = _dot_nt(dg_s[r, :], z2n_s[...]).astype(BF)
            cp1(i).start()
            dz2n = _r(_dot_tn(wsp_ref[:, r], dg_s[...]))
            z, gp = _gelu_and_grad(pre_s[r, FH:].astype(F32))
            xh, sd = _ln(_r(z))
            pre_s[r, FH:] = (_ln_bwd(dz2n, xh, sd) * gp).astype(BF)
            dhn = _dot_nt(pre_s[r, :], win_ref[...])
            hh, hsd = _ln(h_s[r, :].astype(F32))
            h_s[r, :] = (_r(go_ref[r, :].astype(F32) + _ln_bwd(dhn, hh, hsd))).astype(BF)
            return c
        lax.fori_loop(0, NT, b1, 0)
        cp1(NT - 2).wait()
        cp1(NT - 1).wait()

        def b2(i, c):
            cs = pl.ds(pl.multiple_of(i * 512, 512), 512)

            @pl.when(i >= 2)
            def _():
                cp2(i - 2).wait()
            buf2[i % 2] = _dot_tn(dx_ref[...], pre_s[:, cs]).astype(BF)
            cp2(i).start()
            return c
        n2 = 2 * FH // 512
        lax.fori_loop(0, n2, b2, 0)
        cp2(n2 - 2).wait()
        cp2(n2 - 1).wait()

    FF = win_ref.shape[1]
    pl.run_scoped(gmlp, pltpu.VMEM((L, FF), BF),
                  pltpu.VMEM((L, FF // 2), BF), pltpu.VMEM((L, FF // 2), BF),
                  pltpu.VMEM((FF // 2, D), F32), pltpu.VMEM((2, TM, L), BF), pltpu.VMEM((2, D, 512), BF),
                  pltpu.SemaphoreType.DMA((2,)), pltpu.SemaphoreType.DMA((2,)))


    def ssm_bwd(dw_s):
        def tr2(a, c):
            dh = h_s[pl.ds(a * C, C), :].astype(F32)
            dw_s[a] = _dot3(fh, fl, dh)
            return c + jnp.sum(dh * xn_s[pl.ds(a * C, C), :].astype(F32), axis=0, keepdims=True)
        ddsk_ref[...] = lax.fori_loop(0, NB, tr2, jnp.zeros((1, D), F32)).astype(BF)

        def win(a, c):
            ap = jnp.minimum(a + 1, NB - 1)
            w = jnp.where(a + 1 < NB, 1.0, 0.0) * sgn
            nr = dw_s[a, :C, :] + w * dw_s[ap, C:, :]
            ni = dw_s[a, C:, :] - w * dw_s[ap, :C, :]
            dw_s[a, :C, :] = nr
            dw_s[a, C:, :] = ni
            return c
        lax.fori_loop(0, NB, win, 0)

        def bconv(a, c):
            acc = [[], [], [], []]
            for k0 in range(0, C, 16):
                re = slice(k0, k0 + 16); im = slice(C + k0, C + k0 + 16)

                def inner(dl, cc):
                    gr, gi, kr_, ki_ = cc
                    wr_ = dw_s[a + dl, re, :]; wi_ = dw_s[a + dl, im, :]
                    kr = kf_s[dl, re, :]; ki = kf_s[dl, im, :]
                    ur = u_s[dl, re, :]; ui = u_s[dl, im, :]
                    return (gr + kr * wr_ + ki * wi_, gi + kr * wi_ - ki * wr_,
                            kr_ + ur * wr_ + ui * wi_, ki_ + ur * wi_ - ui * wr_)
                z0 = jnp.zeros((16, D), F32)
                for lst, v in zip(acc, lax.fori_loop(0, NB - a, inner, (z0, z0, z0, z0))):
                    lst.append(v)
            r = pl.ds(a * C, C)
            du = _dot3(fth, ftl, jnp.concatenate(acc[0] + acc[1], axis=0))
            k_s[r, :] = _dot3(fth, ftl, jnp.concatenate(acc[2] + acc[3], axis=0))
            dh = h_s[r, :].astype(F32)
            dxn = du + dh * dsk_ref[...].astype(F32)
            xh, sd = _ln(x_ref[r, :].astype(F32))
            dx_ref[r, :] = (dh + _ln_bwd(dxn, xh, sd)).astype(BF)
            return c
        lax.fori_loop(0, NB, bconv, 0)

    pl.run_scoped(ssm_bwd, pltpu.VMEM((NB, 2 * C, D), F32))

    kd_s[...] = jnp.zeros(kd_s.shape, F32)

    def kred(i, c):
        q0 = qwin(i)
        q = q0 + lax.broadcasted_iota(jnp.int32, (256, C), 0)
        l = i * C + lax.broadcasted_iota(jnp.int32, (256, C), 1)
        kd_s[pl.ds(q0, 256), :] += _dot_sel(jnp.where(_l_to_q(l) == q, 1.0, 0.0).astype(BF),
                                            k_s[pl.ds(i * C, C), :])
        return c
    lax.fori_loop(0, NB, kred, 0)

    def pgrad(lo_s, st_s):
        outs = (dare_ref, daim_ref, dbre_ref, dbim_ref)

        def chunk(nc, c0):
            rn = pl.ds(pl.multiple_of(nc * 16, 16), 16)
            fill_lo(lo_s, rn)
            z = jnp.zeros((16, D), F32)
            for o in outs:
                o[rn, :] = z
            for sg, (j0, j1) in enumerate(SEG):
                st_s[0], st_s[1] = cexp(float((0, 256, 512, 1024)[sg]), rn)
                st_s[2], st_s[3] = cexp(float(8 << sg), rn)

                def pg(j, c):
                    t1r = t1i = t2r = t2i = z
                    for b in range(8):
                        d1 = kd_s[pl.ds(8 * j + b, 1), :]
                        d2 = d1 * float(b << sg)
                        lr = lo_s[0, 8 * sg + b]; li = lo_s[1, 8 * sg + b]
                        t1r = t1r + d1 * lr; t1i = t1i + d1 * li
                        t2r = t2r + d2 * lr; t2i = t2i + d2 * li
                    rh = _q_to_r(8 * j).astype(F32)
                    t2r = t2r + rh * t1r; t2i = t2i + rh * t1i
                    hr = st_s[0]; hi = st_s[1]
                    dare_ref[rn, :] += hr * t1r - hi * t1i
                    daim_ref[rn, :] += hr * t1i + hi * t1r
                    dbre_ref[rn, :] += hr * t2r - hi * t2i
                    dbim_ref[rn, :] += hr * t2i + hi * t2r
                    sr = st_s[2]; si = st_s[3]
                    st_s[0] = hr * sr - hi * si
                    st_s[1] = hr * si + hi * sr
                    return c
                lax.fori_loop(j0, j1, pg, 0)
            return c0
        lax.fori_loop(0, N // 16, chunk, 0)
        g = (dare_ref[...], daim_ref[...], dbre_ref[...], dbim_ref[...])
        g1r, g1i, g2r, g2i = g
        wr, wi = wmat()
        br = bre_ref[...] * dt; bi = bim_ref[...] * dt
        cr = cre_ref[...]; ci = cim_ref[...]
        gwr, gwi = g1r, -g1i
        glr = wr * g2r - wi * g2i
        gli = -(wr * g2i + wi * g2r)
        gbr = gwr * cr + gwi * ci; gbi = gwi * cr - gwr * ci
        dcre_ref[...] = gwr * br + gwi * bi; dcim_ref[...] = gwi * br - gwr * bi
        dbre_ref[...] = gbr * dt; dbim_ref[...] = gbi * dt
        dare_ref[...] = glr * dt; daim_ref[...] = gli * dt
        dldt_ref[...] = jnp.sum(gbr * br + gbi * bi + dt * (glr * are_ref[...] + gli * aim_ref[...]),
                                axis=0, keepdims=True).astype(BF)
    pl.run_scoped(pgrad, pltpu.VMEM((2, 32, 16, D), F32), pltpu.VMEM((4, 16, D), F32))
    for k_, r_ in enumerate((o0, o1, o2, o3, o4, o5)):
        r_[...] = pout_s[k_].T.astype(BF)


@jax.jit
def pallas_sequential_preLN__ssm_conv_s4__mixer_gmlp__prompt_kernel(
    A_u, A_A_re, A_A_im, A_B_re, A_B_im, A_C_re, A_C_im, A_log_dt, A_Dskip,
    B_x, B_w_in, B_w_sp, B_b_sp, B_w_out, grad_out,
):
    _, L, D = A_u.shape
    N = A_A_re.shape[1]
    F = B_w_in.shape[1]
    FH = F // 2
    S = jax.ShapeDtypeStruct
    nd = S((D, N), BF)
    V = pl.BlockSpec(memory_space=pltpu.VMEM)
    H = pl.BlockSpec(memory_space=pl.ANY)
    outs = pl.pallas_call(
        _kernel,
        out_shape=(S((L, D), BF), S((L, D), BF), nd, nd, nd, nd, nd, nd, S((1, D), BF), S((1, D), BF),
                   S((D, F), BF), S((L, L), BF), S((L, 1), BF), S((FH, D), BF)),
        in_specs=[V] * 9 + [H, H, V, H, H],
        out_specs=tuple([V] * 10 + [H, H, V, V]),
        scratch_shapes=[
            pltpu.VMEM((L, D), BF), pltpu.VMEM((L, D), BF),
            pltpu.VMEM((L, D), F32), pltpu.VMEM((QP, D), F32),
            pltpu.VMEM((L // C, 2 * C, D), F32), pltpu.VMEM((L // C, 2 * C, D), F32),
            pltpu.VMEM((D, F), BF), pltpu.VMEM((L, L), BF), pltpu.VMEM((FH, D), BF),
            pltpu.VMEM((L, D), BF), pltpu.SemaphoreType.DMA((4,)),
            pltpu.VMEM((6, N, D), F32), pltpu.VMEM((6, N, D), F32),
        ],
        compiler_params=pltpu.CompilerParams(vmem_limit_bytes=127 * 1024 * 1024),
    )(A_u[0], A_A_re, A_A_im, A_B_re, A_B_im, A_C_re, A_C_im,
      A_log_dt.reshape(1, D), A_Dskip.reshape(1, D), B_w_in, B_w_sp, B_b_sp.reshape(L, 1),
      B_w_out, grad_out[0])
    o, dx, a1, a2, b1, b2, c1, c2, dl, dd, dwi, dws, dbs, dwo = outs
    return (o[None], dx[None], a1, a2, b1, b2, c1, c2, dl.reshape(D), dd.reshape(D),
            dwi, dws, dbs.reshape(L), dwo)
```
